```python
import os as _os
_os.environ.setdefault("JAX_PLATFORMS", "cpu")
import jax
import jax.numpy as jnp

def _softmax(x, axis=-1):
    return jax.nn.softmax(x, axis=axis)
def _gelu(x):
    return jax.nn.gelu(x, approximate=True)
def _silu(x):
    return jax.nn.silu(x)
def _sigmoid(x):
    return jax.nn.sigmoid(x)
def _layernorm(x, axis=-1, eps=1e-5):
    m = jnp.mean(x, axis=axis, keepdims=True)
    v = jnp.var(x, axis=axis, keepdims=True)
    return (x - m) / jnp.sqrt(v + eps)
def _scatter_add(tgt, idx, src, axis=0):
    return tgt.at[idx].add(src)
def _segment_sum(src, seg, n):
    return jax.ops.segment_sum(src, seg, n)
class _Rng:
    def __init__(self, key):
        self._k = key
    def _next(self):
        self._k, sub = jax.random.split(self._k)
        return sub
    def normal(self, shape):
        return jax.random.normal(self._next(), shape, dtype=jnp.bfloat16)
    def randint(self, lo, hi, shape):
        return jax.random.randint(self._next(), shape, lo, hi, dtype=jnp.int32)
    def uniform(self, shape, lo=0.0, hi=1.0):
        return jax.random.uniform(self._next(), shape, jnp.bfloat16, lo, hi)
    def permutation(self, n):
        return jax.random.permutation(self._next(), n)


kernel_name = 'gated_mix__mha_block__mixer_s_mlp__prompt'

def setup_inputs():
    _rng = _Rng(jax.random.key(int.from_bytes(__import__("os").urandom(4), "little")))
    _w = (lambda a: (lambda t: t.astype(jnp.bfloat16) if jnp.issubdtype(t.dtype, jnp.floating) else t)(jnp.asarray(a)))
    def _A_setup():
        B, S, D, H = 1, 2048, 448, 16
        return {
            "x": _w((lambda *s: _rng.normal(s) * 0.05)(B, S, D)),
            "wqkv": _w((lambda *s: _rng.normal(s) * 0.8)(D, 3 * D)),
            "wo": _w((lambda *s: _rng.normal(s) * 0.05)(D, D)),
        }
    _A_in = _A_setup()

    def _B_setup():
        B, S, D, F = 1, 2048, 448, 1792
        return {
            "x":  _w((lambda *s: _rng.normal(s) * 0.05)(B, S, D)),
            "w1": _w((lambda *s: _rng.normal(s) * 0.2)(D, D) * (D ** -0.5)),
            "w2": _w((lambda *s: _rng.normal(s) * 0.2)(D, D) * (D ** -0.5)),
            "w3": _w((lambda *s: _rng.normal(s) * 0.2)(D, F) * (D ** -0.5)),
            "w4": _w((lambda *s: _rng.normal(s) * 0.2)(F, D) * (F ** -0.5)),
        }
    _B_in = _B_setup()

    return {
        "A_x": _A_in["x"],
        "A_wqkv": _A_in["wqkv"],
        "A_wo": _A_in["wo"],
        "B_x": _B_in["x"],
        "B_w1": _B_in["w1"],
        "B_w2": _B_in["w2"],
        "B_w3": _B_in["w3"],
        "B_w4": _B_in["w4"],
        "gate_w": _w((lambda *s: _rng.normal(s) * 0.05)(448) * 16.0),
    }

def reference(A_x, A_wqkv, A_wo, B_x, B_w1, B_w2, B_w3, B_w4, gate_w):
    def _A_ref(x, wqkv, wo):
        B, S, D = x.shape
        H = 16
        Dh = D // H
        qkv = (lambda x, *d: x.transpose(*d))((x @ wqkv).reshape(B, S, 3, H, Dh), 2, 0, 3, 1, 4)
        q, k, v = qkv[0], qkv[1], qkv[2]
        scores = jnp.einsum("bhqd,bhkd->bhqk", q, k) * (Dh ** -0.5)
        p = _softmax(scores, axis=-1)
        o = jnp.einsum("bhqk,bhkd->bhqd", p, v)
        return (lambda x, *d: x.transpose(*d))(o, 0, 2, 1, 3).reshape(B, S, D) @ wo

    def _B_ref(x, w1, w2, w3, w4):
        B, S, D = x.shape
        h = _gelu(_layernorm(x, axis=-1) @ w1)
        c = D // 4
        g0 = jnp.pad(h[:, :, 0*c:1*c], ((0, 0), (1, 0), (0, 0)))[:, :S, :]
        g1 = jnp.pad(h[:, :, 1*c:2*c], ((0, 0), (0, 1), (0, 0)))[:, 1:, :]
        g2 = jnp.pad(h[:, :, 2*c:3*c], ((0, 0), (2, 0), (0, 0)))[:, :S, :]
        g3 = jnp.pad(h[:, :, 3*c:   ], ((0, 0), (0, 2), (0, 0)))[:, 2:, :]
        hs = jnp.concatenate([g0, g1, g2, g3], axis=-1) @ w2
        x1 = x + hs
        h2 = _gelu(_layernorm(x1, axis=-1) @ w3) @ w4
        return x1 + h2

    x = A_x
    g = _sigmoid((x * gate_w).sum(-1, keepdims=True))
    a = _A_ref(x, A_wqkv, A_wo)
    b = _B_ref(x, B_w1, B_w2, B_w3, B_w4)
    return g * a + (1 - g) * b
```

```python
import functools, math, os
import jax
import jax.numpy as jnp
import jax.experimental.pallas as pl
import jax.experimental.pallas.tpu as pltpu

S, D, H, DH, F = 2048, 448, 16, 28, 1792
HP = 32
DP = H * HP
GR = 4 * DH
TQ = 256
NB = S // TQ
KC = int(os.environ.get("KC", 128))
SMV = os.environ.get("SMV", "B")
MI = int(os.environ.get("MI", 1))
FC = int(os.environ.get("FC", 128))
DC = int(os.environ.get("DC", 128))
DL = int(os.environ.get("DL", 1))
LAG = int(os.environ.get("LAG", 0))
NK = S // KC
C = D // 4
EPS = 1e-5
QSCALE = (DH ** -0.5) * math.log2(math.e)
HALO = 128
f32, bf16 = jnp.float32, jnp.bfloat16


def _gelu(x):
    c = math.sqrt(2.0 / math.pi)
    return 0.5 * x * (1.0 + jnp.tanh(c * (x + 0.044715 * (x * x * x))))


def _lnT(x):
    m = jnp.mean(x, axis=0, keepdims=True)
    xc = x - m
    v = jnp.mean(xc * xc, axis=0, keepdims=True)
    return xc * jax.lax.rsqrt(v + EPS)


def _dot(a, b):
    return jnp.dot(a, b, preferred_element_type=f32)


def kernel(x_hbm, wqkv_hbm, wo_hbm, w1_hbm, w2_hbm, w3_hbm, w4T_hbm, gw_hbm,
           o_ref,
           x_s, wqkv_r, wo_r, w1_r, w2_r, w3_r, w4T_s, gw_r,
           wqkvT_s, woT_s, w1T_s, w2T_s, w3T_s, wop_s,
           k_s, vT_s, ln1_s, h_s, hs_s, g_s, sA, sB, q_s, oT_s, sems):
    i = pl.program_id(0)

    @pl.when(i == 0)
    def _prologue():
        cp = pltpu.make_async_copy
        cx = [cp(x_hbm.at[:, pl.ds(b * TQ, TQ)], x_s.at[b], sems.at[b]) for b in range(NB)]
        c_wk = cp(wqkv_hbm.at[:, pl.ds(384, 512)], wqkv_r.at[:, pl.ds(384, 512)], sems.at[8])
        c_wv = cp(wqkv_hbm.at[:, pl.ds(896, 448)], wqkv_r.at[:, pl.ds(896, 448)], sems.at[9])
        c_wq = cp(wqkv_hbm.at[:, pl.ds(0, 384)], wqkv_r.at[:, pl.ds(0, 384)], sems.at[10])
        c_gw = cp(gw_hbm, gw_r, sems.at[11])
        c_w1 = cp(w1_hbm, w1_r, sems.at[12])
        c_w2 = cp(w2_hbm, w2_r, sems.at[13])
        c_wo = cp(wo_hbm, wo_r, sems.at[14])
        c_w3 = cp(w3_hbm, w3_r, sems.at[15])
        c_w4 = cp(w4T_hbm, w4T_s, sems.at[16])
        for c in [c_wk] + cx + [c_wv, c_gw, c_w1, c_wq, c_w2, c_wo, c_w3, c_w4]:
            c.start()

        h_s[:, 0:HALO] = jnp.zeros((D, HALO), bf16)
        h_s[:, HALO + S:] = jnp.zeros((D, HALO), bf16)
        wop_s[...] = jnp.zeros(wop_s.shape, f32)

        def kproj(b):
            xb = x_s[b]
            kT = _dot(wqkvT_s[D:2 * D, :], xb).astype(bf16)
            for g in range(4):
                k_s[g, b * TQ:(b + 1) * TQ, :] = kT[g * GR:(g + 1) * GR, :].T
            ln1_s[b] = _lnT(xb.astype(f32)).astype(bf16)

        c_wk.wait()
        wqkvT_s[384:896, :] = wqkv_r[:, 384:896].T
        cx[0].wait(); cx[1].wait()
        kproj(0); kproj(1)
        for b in range(2, 6):
            cx[b].wait()
        for b in range(2, 6):
            kproj(b)
        cx[6].wait(); cx[7].wait(); c_wv.wait(); c_gw.wait(); c_w1.wait(); c_wq.wait()
        w1T_s[...] = w1_r[...].T
        kproj(6); kproj(7)
        wqkvT_s[896:3 * D, :] = wqkv_r[:, 896:3 * D].T
        wqkvT_s[3 * D:, :] = jnp.broadcast_to(gw_r[...].reshape(1, D), (16, D))
        wqkvT_s[0:384, :] = wqkv_r[:, 0:384].T
        for b in range(NB):
            h_s[:, HALO + b * TQ:HALO + (b + 1) * TQ] = _gelu(_dot(w1T_s[...], ln1_s[b])).astype(bf16)

        c_w2.wait(); c_wo.wait(); c_w3.wait(); c_w4.wait()
        w2T_s[...] = w2_r[...].T
        wof = wo_r[...].astype(f32)
        for h in range(H):
            wop_s[h * HP:h * HP + DH, :] = wof[h * DH:(h + 1) * DH, :]
        woT_s[...] = wop_s[...].astype(bf16).T
        w3T_s[...] = w3_r[...].T

        row = jax.lax.broadcasted_iota(jnp.int32, (HP, TQ), 0)
        pad_rows = jnp.where(row == DH, 1.0, 0.0)
        for b in range(NB):
            cols = slice(b * TQ, (b + 1) * TQ)
            vg = _dot(wqkvT_s[2 * D:, :], x_s[b])
            for h in range(H):
                vT_s[h * HP:(h + 1) * HP, cols] = jnp.where(
                    row < DH, vg[h * DH:h * DH + HP, :], pad_rows).astype(bf16)
            g_s[b] = jax.nn.sigmoid(vg[D:D + 8, :])
            l0 = HALO + b * TQ
            for g, off in enumerate((-1, 1, -2, 2)):
                hs_s[b, g * C:(g + 1) * C, :] = h_s[g * C:(g + 1) * C, l0 + off:l0 + off + TQ]

    zi = jnp.minimum(i, 0)
    xb = x_s[i]
    q_s[...] = (_dot(wqkvT_s[0:D, :], xb) * QSCALE).astype(bf16)
    x1 = xb.astype(f32) + _dot(w2T_s[...], hs_s[i])
    ln2 = _lnT(x1).astype(bf16)

    grow = jax.lax.broadcasted_iota(jnp.int32, (GR, TQ), 0)
    sbuf = (sA, sB)
    NP = H // 2
    qm = [None] * NP
    pmax = [None] * NP
    mx = [None] * NP
    acc = [None] * H
    gch = [None] * (F // FC)
    st = {"b": x1}

    def qk(p, c):
        g = p // 2
        if c == 0:
            qg = q_s[g * GR:(g + 1) * GR, :]
            z = jnp.zeros_like(qg)
            j = (2 * p) % 4
            qm[p] = jnp.concatenate(
                [jnp.where((grow >= jj * DH) & (grow < (jj + 1) * DH), qg, z) for jj in (j, j + 1)], axis=1)
        s = _dot(k_s[g, c * KC:(c + 1) * KC, :], qm[p])
        sbuf[p % 2][zi, c * KC:(c + 1) * KC, :] = s
        pm = jnp.max(s.reshape(KC // 8, 8, 2 * TQ), axis=0)
        pmax[p] = pm if c == 0 else jnp.maximum(pmax[p], pm)
        if c == NK - 1:
            mx[p] = jnp.max(pmax[p], axis=0, keepdims=True)

    def fin(h):
        oT_s[h * HP:(h + 1) * HP, :] = (acc[h] * (1.0 / acc[h][DH:DH + 1, :])).astype(bf16)

    def smA(p, c):
        pp = jnp.exp2(sbuf[p % 2][zi, c * KC:(c + 1) * KC, :] - mx[p]).astype(bf16)
        for e in range(2):
            h = 2 * p + e
            d = _dot(vT_s[h * HP:(h + 1) * HP, c * KC:(c + 1) * KC], pp[:, e * TQ:(e + 1) * TQ])
            acc[h] = d if c == 0 else acc[h] + d
            if c == NK - 1:
                fin(h)

    def smB(p, c):
        e, cc = c % 2, c // 2
        h = 2 * p + e
        pp = jnp.exp2(sbuf[p % 2][zi, cc * 2 * KC:(cc + 1) * 2 * KC, e * TQ:(e + 1) * TQ]
                      - mx[p][:, e * TQ:(e + 1) * TQ]).astype(bf16)
        d = _dot(vT_s[h * HP:(h + 1) * HP, cc * 2 * KC:(cc + 1) * 2 * KC], pp)
        acc[h] = d if cc == 0 else acc[h] + d
        if cc == NK // 2 - 1:
            fin(h)

    sm = smA if SMV == "A" else smB

    nf = F // FC

    R = DC // FC

    def up(c):
        gch[c] = _gelu(_dot(w3T_s[c * FC:(c + 1) * FC, :], ln2)).astype(bf16)

    def down(c):
        gg = gch[c] if R == 1 else jnp.concatenate(gch[c * R:(c + 1) * R], axis=0)
        st["b"] = st["b"] + _dot(w4T_s[:, c * DC:(c + 1) * DC], gg)

    def oproj(_):
        st["a"] = _dot(woT_s[...], oT_s[...])

    dots = []
    nd = F // DC
    for c in range(nf):
        dots.append((up, c))
        d = (c + 1 - DL) // R - 1
        if (c + 1 - DL) % R == 0 and d >= 0:
            dots.append((down, d))
    rest = [d for d in range(nd) if (down, d) not in dots]
    dots += [(oproj, 0)] + [(down, d) for d in rest]

    for n in range(NP * NK):
        qk(n // NK, n % NK)
        m = n - NK - LAG
        if m >= 0:
            sm(m // NK, m % NK)
    m = NP * NK - NK - LAG
    for fn, c in dots:
        if fn is oproj:
            assert m == NP * NK
        fn(c)
        for _ in range(MI):
            if m < NP * NK:
                sm(m // NK, m % NK)
                m += 1
    a = st["a"]
    gt = g_s[i, 0:1, :]
    o_ref[...] = (gt * a + (1.0 - gt) * st["b"]).astype(o_ref.dtype)


@jax.jit
def pallas_gated_mix__mha_block__mixer_s_mlp__prompt_kernel(A_x, A_wqkv, A_wo, B_x, B_w1, B_w2, B_w3, B_w4, gate_w):
    xT = A_x.reshape(S, D).T
    args = (xT, A_wqkv, A_wo, B_w1, B_w2, B_w3, B_w4.T, gate_w)
    V = pltpu.VMEM
    outT = pl.pallas_call(
        kernel,
        grid=(NB,),
        in_specs=[pl.BlockSpec(memory_space=pl.ANY)] * len(args),
        out_specs=pl.BlockSpec((D, TQ), lambda i: (0, i)),
        out_shape=jax.ShapeDtypeStruct((D, S), bf16),
        scratch_shapes=[
            V((NB, D, TQ), bf16),
            V((D, 3 * D), bf16),
            V((D, D), bf16),
            V((D, D), bf16),
            V((D, D), bf16),
            V((D, F), bf16),
            V((D, F), bf16),
            V((D,), bf16),
            V((3 * D + 16, D), bf16),
            V((D, DP), bf16),
            V((D, D), bf16),
            V((D, D), bf16),
            V((F, D), bf16),
            V((DP, D), f32),
            V((4, S, GR), bf16),
            V((DP, S), bf16),
            V((NB, D, TQ), bf16),
            V((D, S + 2 * HALO), bf16),
            V((NB, D, TQ), bf16),
            V((NB, 8, TQ), f32),
            V((1, S, 2 * TQ), f32),
            V((1, S, 2 * TQ), f32),
            V((D, TQ), bf16),
            V((DP, TQ), bf16),
            pltpu.SemaphoreType.DMA((17,)),
        ],
        compiler_params=pltpu.CompilerParams(
            dimension_semantics=("arbitrary",), vmem_limit_bytes=100 * 1024 * 1024),
    )(*args)
    return outT.T.reshape(1, S, D)
```

```python
import functools
import math

import jax
import jax.numpy as jnp
import jax.experimental.pallas as pl
import jax.experimental.pallas.tpu as pltpu

S, D, H, DH, F = 2048, 448, 16, 28, 1792
HP = 32
DP = H * HP
GR = 4 * DH
TQ = 256
NB = S // TQ
KC = 128
NK = S // KC
NP = H // 2
FH, D2, DP2 = F // 2, D // 2, DP // 2
NC = FH // 128
C = D // 4
HALO = 128
EPS = 1e-5
QSCALE = (DH ** -0.5) * math.log2(math.e)
f32, bf16 = jnp.float32, jnp.bfloat16

SDPOS = {2: (0, 0), 3: (D2, FH), 0: (D, 0), 1: (D, FH), 4: (D + D2, 0), 5: (D + D2, FH), 6: (2 * D, 0)}
PLAN = [
    ("g wk", "Twk Tg"),
    ("x0 x1", "K0 S0 K1 S1"),
    ("x2 x3 x4 x5", "K2 S2 T0 K3 S3 T1 K4 S4 K5 S5"),
    ("x6 x7 w1 wv wq", "Tw1 K6 S6 K7 S7 Twv Twq W0 T2 W6 T3 W7 T4 W1 T5 W2 T6 W3 T7 W4 W5"),
    ("w2 wo w3 w4", "Tw2 Two Tw3 Tw4 V0 H0 V1 H1 V2 H2 V3 H3 V4 H4 V5 H5 V6 H6 V7 H7"),
]
SCRATCH = dict(
    sA=((1, S, 2 * TQ), f32), sB=((1, S, 2 * TQ), f32), k_s=((4, S, GR), bf16), vT_s=((DP, S), bf16),
    x_s=((NB, D, TQ), bf16), wqkv_r=((D, 3 * D), bf16), wo_r=((D, D), bf16), w1_r=((D, D), bf16),
    w2_r=((D, D), bf16), w3_r=((D, F), bf16), w4_s=((D + 3 * D2, F), bf16), gw_r=((D,), bf16),
    wqkvT_s=((3 * D, D), bf16), so_s=((7, D2, DP2), bf16), w1T_s=((D, D), bf16),
    s2_s=((7, D2, D2), bf16), s3_s=((7, FH, D2), bf16), wop_s=((DP, D), f32), gcol_s=((D, 128), f32),
    scol_s=((D, 128), f32), kT_s=((NB, D, TQ), bf16), st_s=((NB, 8, TQ), f32),
    h_s=((D, S + 2 * HALO), bf16), hs_s=((NB, D, TQ), bf16), q_s=((D, TQ), bf16), oT_s=((DP, TQ), f32),
    oa_s=((NB, 2, C, TQ), bf16), ob_s=((NB, 2, C, TQ), bf16), x1_s=((1, D + 16, TQ), f32),
    sb_s=((1, D2, 7 * 128), bf16))


def _gelu(x, half=0.5):
    c = math.sqrt(2.0 / math.pi)
    return half * x * (1.0 + jnp.tanh(c * (x + 0.044715 * (x * x * x))))


def _dot(a, b):
    return jnp.dot(a, b, preferred_element_type=f32)


def _ln_stats(x):
    c0 = x[0:1, :]
    d = x - c0
    m1 = jnp.mean(d, axis=0, keepdims=True)
    m2 = jnp.mean(d * d, axis=0, keepdims=True)
    return c0 + m1, jax.lax.rsqrt(jnp.maximum(m2 - m1 * m1, 0.0) + EPS)


def _sa(a11, a12, a21, a22):
    return [a11 + a22, a21 + a22, a11, a22, a11 + a12, a21 - a11, a12 - a22]


def _sb(b11, b12, b21, b22):
    return [t.astype(bf16) for t in (b11 + b22, b11, b12 - b22, b21 - b11, b22, b11 + b12, b21 + b22)]


def _sc(m):
    return m[0] + m[3] - m[4] + m[6], m[2] + m[4], m[1] + m[3], m[0] - m[1] + m[2] + m[5]


def _quad(x):
    r = x.shape[0] // 2
    return x[:r, :128], x[:r, 128:], x[r:, :128], x[r:, 128:]


def _col(row):
    return jnp.broadcast_to(row, (128, D)).T


def _wide(col):
    return jnp.concatenate([col] * (TQ // 128), axis=1)


def _kernel(x_hbm, wqkv_hbm, wo_hbm, w1_hbm, w2_hbm, w3_hbm, w4T_hbm, gw_hbm, o_hbm,
            sA, sB, k_s, vT_s, x_s, wqkv_r, wo_r, w1_r, w2_r, w3_r, w4_s, gw_r, wqkvT_s, so_s, w1T_s,
            s2_s, s3_s, wop_s, gcol_s, scol_s, kT_s, st_s, h_s, hs_s, q_s, oT_s, oa_s, ob_s, x1_s, sb_s,
            sems, osems):
    i = pl.program_id(0)
    zi = jnp.minimum(i, 0)
    cp = pltpu.make_async_copy

    @pl.when(i == 0)
    def _prologue():
        row = jax.lax.broadcasted_iota(jnp.int32, (HP - DH, TQ), 0)
        pad_rows = jnp.where(row == 0, 1.0, 0.0)

        def kproj(b):
            kT_s[b] = _dot(wqkvT_s[D:2 * D, :], x_s[b]).astype(bf16)

        def ktr(b):
            for g in range(4):
                k_s[g, b * TQ:(b + 1) * TQ, :] = kT_s[b, g * GR:(g + 1) * GR, :].T

        def stats(b):
            xf = x_s[b].astype(f32)
            mu, rstd = _ln_stats(xf)
            z = jnp.sum(xf * _wide(gcol_s[...]), axis=0, keepdims=True)
            st_s[b, 0:1, :] = rstd
            st_s[b, 1:2, :] = mu * rstd
            st_s[b, 2:3, :] = jax.nn.sigmoid(z)

        def w1proj(b):
            y = _dot(w1T_s[...], x_s[b])
            pre = y * st_s[b, 0:1, :] - _wide(scol_s[...]) * st_s[b, 1:2, :]
            h_s[:, HALO + b * TQ:HALO + (b + 1) * TQ] = _gelu(pre).astype(bf16)

        def vproj(b):
            v = _dot(wqkvT_s[2 * D:, :], x_s[b])
            for h in range(H):
                vT_s[h * HP:(h + 1) * HP, b * TQ:(b + 1) * TQ] = jnp.concatenate(
                    [v[h * DH:(h + 1) * DH, :], pad_rows], axis=0).astype(bf16)

        def shift(b):
            l0 = HALO + b * TQ
            for g, off in enumerate((-1, 1, -2, 2)):
                hs_s[b, g * C:(g + 1) * C, :] = h_s[g * C:(g + 1) * C, l0 + off:l0 + off + TQ]

        def t_qkv(lo, hi):
            wqkvT_s[lo:hi, :] = wqkv_r[:, lo:hi].T

        def t_w1():
            w1T_s[...] = w1_r[...].T
            scol_s[...] = _col(jnp.sum(w1_r[...].astype(f32), axis=0, keepdims=True))

        def left_ops(w, dst):
            kh = w.shape[0] // 2
            t1, t2 = w[:kh].T.astype(f32), w[kh:].T.astype(f32)
            for k, a in enumerate(_sa(t1[:D2], t2[:D2], t1[D2:], t2[D2:])):
                dst[k] = a.astype(bf16)

        def t_wo():
            wof = wo_r[...].astype(f32)
            for h in range(H):
                wop_s[h * HP:h * HP + DH, :] = wof[h * DH:(h + 1) * DH, :]
            left_ops(wop_s[...].astype(bf16), so_s)

        def t_w3():
            for c in range(NC):
                def blk(r, e):
                    return w3_r[r * D2:(r + 1) * D2, e * FH + c * 128:e * FH + (c + 1) * 128].astype(f32)
                for k, a in enumerate(_sa(blk(0, 0), blk(1, 0), blk(0, 1), blk(1, 1))):
                    s3_s[k, c * 128:(c + 1) * 128, :] = a.astype(bf16).T

        def t_w4():
            for r0 in range(0, D2, 16):
                def rows(base):
                    return pl.ds(pl.multiple_of(zi * 16 + base + r0, 16), 16)
                for c0 in range(0, FH, 256):
                    c1 = min(c0 + 256, FH)
                    def blk(r, e):
                        return w4_s[rows(r * D2), e * FH + c0:e * FH + c1].astype(f32)
                    for k, a in enumerate(_sa(blk(0, 0), blk(0, 1), blk(1, 0), blk(1, 1))):
                        if k not in (2, 3):
                            rb, cb = SDPOS[k]
                            w4_s[rows(rb), cb + c0:cb + c1] = a.astype(bf16)

        def t_g():
            gcol_s[...] = _col(gw_r[...].astype(f32).reshape(1, D))

        def cols(lo, n):
            return wqkv_hbm.at[:, pl.ds(lo, n)], wqkv_r.at[:, pl.ds(lo, n)]

        copies = {"g": (gw_hbm, gw_r), "wk": cols(384, 512), "wv": cols(896, 448), "wq": cols(0, 384),
                  "w1": (w1_hbm, w1_r), "w2": (w2_hbm, w2_r), "wo": (wo_hbm, wo_r), "w3": (w3_hbm, w3_r),
                  "w4": (w4T_hbm, w4_s.at[pl.ds(0, D), :])}
        jobs = {"Twk": functools.partial(t_qkv, 384, 896), "Twv": functools.partial(t_qkv, 896, 3 * D),
                "Twq": functools.partial(t_qkv, 0, 384), "Tw1": t_w1,
                "Tw2": lambda: left_ops(w2_r[...], s2_s), "Two": t_wo, "Tw3": t_w3, "Tw4": t_w4, "Tg": t_g}
        for b in range(NB):
            copies["x%d" % b] = (x_hbm.at[:, pl.ds(b * TQ, TQ)], x_s.at[b])
            for nm, fn in (("K", kproj), ("T", ktr), ("S", stats), ("W", w1proj), ("V", vproj), ("H", shift)):
                jobs["%s%d" % (nm, b)] = functools.partial(fn, b)

        grp = [[cp(*copies[n], sems.at[k]) for n in g.split()] for k, (g, _) in enumerate(PLAN)]
        for c in grp[0] + grp[1]:
            c.start()
        h_s[:, 0:HALO] = jnp.zeros((D, HALO), bf16)
        h_s[:, HALO + S:] = jnp.zeros((D, HALO), bf16)
        wop_s[...] = jnp.zeros(wop_s.shape, f32)
        for k, (_, js) in enumerate(PLAN):
            for c in grp[k]:
                c.wait()
            if k == 0:
                for g in grp[2:]:
                    for c in g:
                        c.start()
            for j in js.split():
                jobs[j]()

    xb = x_s[i]
    q_s[...] = (_dot(wqkvT_s[0:D, :], xb) * QSCALE).astype(bf16)
    gt = st_s[i, 2:3, :]

    hb = _sb(*_quad(hs_s[i].astype(f32)))
    c11, c12, c21, c22 = _sc([_dot(s2_s[k], hb[k]) for k in range(7)])
    x1 = xb.astype(f32) + jnp.concatenate(
        [jnp.concatenate([c11, c12], axis=1), jnp.concatenate([c21, c22], axis=1)], axis=0)
    x1_s[zi, 0:D, :] = x1
    mu, rstd = _ln_stats(x1)
    mu = jnp.broadcast_to(mu, (16, TQ))
    rstd = jnp.broadcast_to(rstd, (16, TQ))
    for r0 in range(0, D2, 16):
        def ld(base):
            return x1_s[0, pl.ds(pl.multiple_of(zi * 16 + base + r0, 16), 16), :]
        t, b = (ld(0) - mu) * rstd, (ld(D2) - mu) * rstd
        ops = _sb(t[:, :128], t[:, 128:], b[:, :128], b[:, 128:])
        for k in range(7):
            sb_s[zi, r0:r0 + 16, k * 128:(k + 1) * 128] = ops[k]
        x1_s[0, pl.ds(pl.multiple_of(zi * 16 + D + (r0 % 32) // 2, 8), 8), 0:128] = t[:8, :128] + b[:8, 128:]

    grow = jax.lax.broadcasted_iota(jnp.int32, (GR, TQ), 0)
    sbuf = (sA, sB)
    qm, pmax, mx, acc = [None] * NP, [None] * NP, [None] * NP, [None] * H

    def qk(p, c):
        g = p // 2
        if c == 0:
            qg = q_s[g * GR:(g + 1) * GR, :]
            z = jnp.zeros_like(qg)
            j = (2 * p) % 4
            qm[p] = jnp.concatenate(
                [jnp.where((grow >= jj * DH) & (grow < (jj + 1) * DH), qg, z) for jj in (j, j + 1)], axis=1)
        s = _dot(k_s[g, c * KC:(c + 1) * KC, :], qm[p])
        sbuf[p % 2][zi, c * KC:(c + 1) * KC, :] = s
        pm = jnp.max(s.reshape(KC // 8, 8, 2 * TQ), axis=0)
        pmax[p] = pm if c == 0 else jnp.maximum(pmax[p], pm)
        if c == NK - 1:
            mx[p] = jnp.max(pmax[p], axis=0, keepdims=True)

    def sm(p, c):
        e, cc = c % 2, c // 2
        h = 2 * p + e
        rows = slice(cc * 2 * KC, (cc + 1) * 2 * KC)
        pp = jnp.exp2(sbuf[p % 2][zi, rows, e * TQ:(e + 1) * TQ] - mx[p][:, e * TQ:(e + 1) * TQ]).astype(bf16)
        d = _dot(vT_s[h * HP:(h + 1) * HP, rows], pp)
        acc[h] = d if cc == 0 else acc[h] + d
        if cc == NK // 2 - 1:
            oT_s[h * HP:(h + 1) * HP, :] = acc[h] * (1.0 / acc[h][DH:DH + 1, :])

    um = [[None] * 7 for _ in range(NC)]
    tb, dm, last, ob = [None] * NC, [None] * 7, [None] * 7, []
    hg = 0.5 * (1.0 - gt)
    hq = (hg[:, :128], hg[:, 128:]) * 2

    def up(c, k):
        um[c][k] = _dot(s3_s[k, c * 128:(c + 1) * 128, :], sb_s[zi, :, k * 128:(k + 1) * 128])
        if k == 6:
            tb[c] = _sb(*[_gelu(t, hh) for t, hh in zip(_sc(um[c]), hq)])

    def down(c, k):
        rb, cb = SDPOS[k]
        d = _dot(w4_s[rb:rb + D2, cb + c * 128:cb + (c + 1) * 128], tb[c][k])
        if c == NC - 1 and k in (1, 2, 5, 6):
            last[k] = d
        else:
            dm[k] = d if c == 0 else dm[k] + d

    def oproj(_, k):
        if not ob:
            ob.extend(_sb(*_quad(oT_s[...] * gt)))
        dm[k] = dm[k] + _dot(so_s[k], ob[k])

    dots = []
    for c in range(NC):
        dots += [(up, c, k) for k in range(7)]
        if c >= 1:
            dots += [(down, c - 1, k) for k in range(7)]
    dots += [(oproj, 0, k) for k in range(7)]
    dots += [(down, NC - 1, k) for k in (0, 3, 4, 1, 2, 5, 6)]

    for n in range(NP * NK):
        qk(n // NK, n % NK)
        if n >= NK:
            sm(n // NK - 1, n % NK)
    for n, (fn, c, k) in enumerate(dots):
        fn(c, k)
        if n % 3 == 2 and n // 3 < NK:
            sm(NP - 1, n // 3)

    base = [xg + cc for xg, cc in zip(_quad(x1_s[zi, 0:D, :] * (1.0 - gt)), _sc(dm))]
    top = jnp.concatenate([base[0] + last[6], base[1] + last[2]], axis=1).astype(bf16)
    bot = jnp.concatenate([base[2] + last[1], base[3] - last[1] + last[2] + last[5]], axis=1).astype(bf16)
    col0 = pl.multiple_of(i * TQ, TQ)
    for n, buf in enumerate((oa_s, ob_s)):
        buf[i, 0] = top[n * C:(n + 1) * C]
        buf[i, 1] = bot[n * C:(n + 1) * C]
        for e in range(2):
            cp(buf.at[i, e], o_hbm.at[pl.ds(e * D2 + n * C, C), pl.ds(col0, TQ)], osems.at[n]).start()

    @pl.when(i == NB - 1)
    def _drain():
        for n, buf in enumerate((oa_s, ob_s)):
            cp(buf, buf, osems.at[n]).wait()


@jax.jit
def pallas_gated_mix__mha_block__mixer_s_mlp__prompt_kernel(
    A_x: jax.Array,
    A_wqkv: jax.Array,
    A_wo: jax.Array,
    B_x: jax.Array,
    B_w1: jax.Array,
    B_w2: jax.Array,
    B_w3: jax.Array,
    B_w4: jax.Array,
    gate_w: jax.Array,
):
    args = (A_x.reshape(S, D).T, A_wqkv, A_wo, B_w1, B_w2, B_w3, B_w4.T, gate_w)
    out_t = pl.pallas_call(
        _kernel,
        grid=(NB,),
        in_specs=[pl.BlockSpec(memory_space=pl.ANY)] * len(args),
        out_specs=pl.BlockSpec(memory_space=pl.ANY),
        out_shape=jax.ShapeDtypeStruct((D, S), bf16),
        scratch_shapes=[pltpu.VMEM(*v) for v in SCRATCH.values()]
        + [pltpu.SemaphoreType.DMA((len(PLAN),)), pltpu.SemaphoreType.DMA((2,))],
        compiler_params=pltpu.CompilerParams(
            dimension_semantics=("arbitrary",), vmem_limit_bytes=100 * 1024 * 1024,
            disable_bounds_checks=True),
    )(*args)
    return out_t.T.reshape(1, S, D)
```

```python
import functools
import math

import jax
import jax.numpy as jnp
import jax.experimental.pallas as pl
import jax.experimental.pallas.tpu as pltpu

S, D, H, DH, F = 2048, 448, 16, 28, 1792
HP = 32
DP = H * HP
GR = 4 * DH
TQ = 256
NB = S // TQ
KC = 128
NK = S // KC
NP = H // 2
FH, D2, DP2 = F // 2, D // 2, DP // 2
NC = FH // 128
C = D // 4
HALO = 128
EPS = 1e-5
QSCALE = (DH ** -0.5) * math.log2(math.e)
f32, bf16 = jnp.float32, jnp.bfloat16

SDPOS = {2: (0, 0), 3: (D2, FH), 0: (D, 0), 1: (D, FH), 4: (D + D2, 0), 5: (D + D2, FH), 6: (2 * D, 0)}
PLAN = [
    ("g wka", "Twka Tg"),
    ("x0", "Ka0 S0"),
    ("wkb", "Twkb Kb0"),
    ("x1 x2", "K1 S1 K2 S2"),
    ("x3 x4 x5 x6", "K3 S3 T0 K4 S4 T1 K5 S5 S6"),
    ("x7 w1 wv wq", "Tw1 K6 K7 S7 Twv Twq W0 T2 W7 T3 W1 T4 W2 T5 W3 T6 W4 T7 W5 W6"),
    ("w2 wo w3 w4", "Tw2 Two Tw3 Tw4 V0 H0 V1 H1 V2 H2 V3 H3 V4 H4 V5 H5 V6 H6 V7 H7"),
]
SCRATCH = dict(
    sA=((1, S, 2 * TQ), f32), sB=((1, S, 2 * TQ), f32), k_s=((4, S, GR), bf16), vT_s=((DP, S), bf16),
    x_s=((NB, D, TQ), bf16), wqkv_r=((D, 3 * D), bf16), wo_r=((D, D), bf16), w1_r=((D, D), bf16),
    w2_r=((D, D), bf16), w3_r=((D, F), bf16), w4_s=((D + 3 * D2, F), bf16), gw_r=((D,), bf16),
    wqkvT_s=((3 * D, D), bf16), so_s=((7, D2, DP2), bf16), w1T_s=((D, D), bf16),
    s2_s=((7, D2, D2), bf16), s3_s=((7, FH, D2), bf16), wop_s=((DP, D), f32), gcol_s=((D, 128), f32),
    scol_s=((D, 128), f32), kT_s=((NB, D, TQ), bf16), st_s=((NB, 8, TQ), f32),
    h_s=((D, S + 2 * HALO), bf16), hs_s=((NB, D, TQ), bf16), q_s=((D, TQ), bf16), oT_s=((DP, TQ), f32),
    oa_s=((NB, 2, C, TQ), bf16), ob_s=((NB, 2, C, TQ), bf16), x1_s=((1, D + 16, TQ), f32),
    sb_s=((1, D2, 7 * 128), bf16))


def _gelu(x, half=0.5):
    c = math.sqrt(2.0 / math.pi)
    return half * x * (1.0 + jnp.tanh(c * (x + 0.044715 * (x * x * x))))


def _dot(a, b):
    return jnp.dot(a, b, preferred_element_type=f32)


def _ln_stats(x):
    c0 = x[0:1, :]
    d = x - c0
    m1 = jnp.mean(d, axis=0, keepdims=True)
    m2 = jnp.mean(d * d, axis=0, keepdims=True)
    return c0 + m1, jax.lax.rsqrt(jnp.maximum(m2 - m1 * m1, 0.0) + EPS)


def _sa(a11, a12, a21, a22):
    return [a11 + a22, a21 + a22, a11, a22, a11 + a12, a21 - a11, a12 - a22]


def _sb(b11, b12, b21, b22):
    return [t.astype(bf16) for t in (b11 + b22, b11, b12 - b22, b21 - b11, b22, b11 + b12, b21 + b22)]


def _sc(m):
    return m[0] + m[3] - m[4] + m[6], m[2] + m[4], m[1] + m[3], m[0] - m[1] + m[2] + m[5]


def _quad(x):
    r = x.shape[0] // 2
    return x[:r, :128], x[:r, 128:], x[r:, :128], x[r:, 128:]


def _col(row):
    return jnp.broadcast_to(row, (128, D)).T


def _wide(col):
    return jnp.concatenate([col] * (TQ // 128), axis=1)


def _kernel(x_hbm, wqkv_hbm, wo_hbm, w1_hbm, w2_hbm, w3_hbm, w4T_hbm, gw_hbm, o_hbm,
            sA, sB, k_s, vT_s, x_s, wqkv_r, wo_r, w1_r, w2_r, w3_r, w4_s, gw_r, wqkvT_s, so_s, w1T_s,
            s2_s, s3_s, wop_s, gcol_s, scol_s, kT_s, st_s, h_s, hs_s, q_s, oT_s, oa_s, ob_s, x1_s, sb_s,
            sems, osems):
    i = pl.program_id(0)
    zi = jnp.minimum(i, 0)
    cp = pltpu.make_async_copy

    @pl.when(i == 0)
    def _prologue():
        row = jax.lax.broadcasted_iota(jnp.int32, (HP - DH, TQ), 0)
        pad_rows = jnp.where(row == 0, 1.0, 0.0)

        def kproj(b, lo=0, hi=D):
            kT_s[b, lo:hi, :] = _dot(wqkvT_s[D + lo:D + hi, :], x_s[b]).astype(bf16)

        def ktr(b):
            for g in range(4):
                k_s[g, b * TQ:(b + 1) * TQ, :] = kT_s[b, g * GR:(g + 1) * GR, :].T

        def stats(b):
            xf = x_s[b].astype(f32)
            mu, rstd = _ln_stats(xf)
            z = jnp.sum(xf * _wide(gcol_s[...]), axis=0, keepdims=True)
            st_s[b, 0:1, :] = rstd
            st_s[b, 1:2, :] = mu * rstd
            st_s[b, 2:3, :] = jax.nn.sigmoid(z)

        def w1proj(b):
            y = _dot(w1T_s[...], x_s[b])
            pre = y * st_s[b, 0:1, :] - _wide(scol_s[...]) * st_s[b, 1:2, :]
            h_s[:, HALO + b * TQ:HALO + (b + 1) * TQ] = _gelu(pre).astype(bf16)

        def vproj(b):
            v = _dot(wqkvT_s[2 * D:, :], x_s[b])
            for h in range(H):
                vT_s[h * HP:(h + 1) * HP, b * TQ:(b + 1) * TQ] = jnp.concatenate(
                    [v[h * DH:(h + 1) * DH, :], pad_rows], axis=0).astype(bf16)

        def shift(b):
            l0 = HALO + b * TQ
            for g, off in enumerate((-1, 1, -2, 2)):
                hs_s[b, g * C:(g + 1) * C, :] = h_s[g * C:(g + 1) * C, l0 + off:l0 + off + TQ]

        def t_qkv(lo, hi):
            wqkvT_s[lo:hi, :] = wqkv_r[:, lo:hi].T

        def t_w1():
            w1T_s[...] = w1_r[...].T
            scol_s[...] = _col(jnp.sum(w1_r[...].astype(f32), axis=0, keepdims=True))

        def left_ops(w, dst):
            kh = w.shape[0] // 2
            t1, t2 = w[:kh].T.astype(f32), w[kh:].T.astype(f32)
            for k, a in enumerate(_sa(t1[:D2], t2[:D2], t1[D2:], t2[D2:])):
                dst[k] = a.astype(bf16)

        def t_wo():
            wof = wo_r[...].astype(f32)
            for h in range(H):
                wop_s[h * HP:h * HP + DH, :] = wof[h * DH:(h + 1) * DH, :]
            left_ops(wop_s[...].astype(bf16), so_s)

        def t_w3():
            for c in range(NC):
                def blk(r, e):
                    return w3_r[r * D2:(r + 1) * D2, e * FH + c * 128:e * FH + (c + 1) * 128].astype(f32)
                for k, a in enumerate(_sa(blk(0, 0), blk(1, 0), blk(0, 1), blk(1, 1))):
                    s3_s[k, c * 128:(c + 1) * 128, :] = a.astype(bf16).T

        def t_w4():
            for r0 in range(0, D2, 16):
                def rows(base):
                    return pl.ds(pl.multiple_of(zi * 16 + base + r0, 16), 16)
                for c0 in range(0, FH, 256):
                    c1 = min(c0 + 256, FH)
                    def blk(r, e):
                        return w4_s[rows(r * D2), e * FH + c0:e * FH + c1].astype(f32)
                    for k, a in enumerate(_sa(blk(0, 0), blk(0, 1), blk(1, 0), blk(1, 1))):
                        if k not in (2, 3):
                            rb, cb = SDPOS[k]
                            w4_s[rows(rb), cb + c0:cb + c1] = a.astype(bf16)

        def t_g():
            gcol_s[...] = _col(gw_r[...].astype(f32).reshape(1, D))

        def cols(lo, n):
            return wqkv_hbm.at[:, pl.ds(lo, n)], wqkv_r.at[:, pl.ds(lo, n)]

        copies = {"g": (gw_hbm, gw_r), "wka": cols(640, 256), "wkb": cols(384, 256),
                  "wv": cols(896, 448), "wq": cols(0, 384),
                  "w1": (w1_hbm, w1_r), "w2": (w2_hbm, w2_r), "wo": (wo_hbm, wo_r), "w3": (w3_hbm, w3_r),
                  "w4": (w4T_hbm, w4_s.at[pl.ds(0, D), :])}
        jobs = {"Twka": functools.partial(t_qkv, 640, 896), "Twkb": functools.partial(t_qkv, 384, 640),
                "Twv": functools.partial(t_qkv, 896, 3 * D), "Twq": functools.partial(t_qkv, 0, 384),
                "Ka0": functools.partial(kproj, 0, 640 - D, D), "Kb0": functools.partial(kproj, 0, 0, 640 - D),
                "Tw1": t_w1,
                "Tw2": lambda: left_ops(w2_r[...], s2_s), "Two": t_wo, "Tw3": t_w3, "Tw4": t_w4, "Tg": t_g}
        for b in range(NB):
            copies["x%d" % b] = (x_hbm.at[:, pl.ds(b * TQ, TQ)], x_s.at[b])
            for nm, fn in (("K", kproj), ("T", ktr), ("S", stats), ("W", w1proj), ("V", vproj), ("H", shift)):
                jobs["%s%d" % (nm, b)] = functools.partial(fn, b)

        grp = [[cp(*copies[n], sems.at[k]) for n in g.split()] for k, (g, _) in enumerate(PLAN)]
        for g in grp:
            for c in g:
                c.start()
        h_s[:, 0:HALO] = jnp.zeros((D, HALO), bf16)
        h_s[:, HALO + S:] = jnp.zeros((D, HALO), bf16)
        wop_s[...] = jnp.zeros(wop_s.shape, f32)
        for k, (_, js) in enumerate(PLAN):
            for c in grp[k]:
                c.wait()
            for j in js.split():
                jobs[j]()

    xb = x_s[i]
    q_s[...] = (_dot(wqkvT_s[0:D, :], xb) * QSCALE).astype(bf16)
    gt = st_s[i, 2:3, :]

    hb = _sb(*_quad(hs_s[i].astype(f32)))
    c11, c12, c21, c22 = _sc([_dot(s2_s[k], hb[k]) for k in range(7)])
    x1 = xb.astype(f32) + jnp.concatenate(
        [jnp.concatenate([c11, c12], axis=1), jnp.concatenate([c21, c22], axis=1)], axis=0)
    x1_s[zi, 0:D, :] = x1
    mu, rstd = _ln_stats(x1)
    mu = jnp.broadcast_to(mu, (16, TQ))
    rstd = jnp.broadcast_to(rstd, (16, TQ))
    for r0 in range(0, D2, 16):
        def ld(base):
            return x1_s[0, pl.ds(pl.multiple_of(zi * 16 + base + r0, 16), 16), :]
        t, b = (ld(0) - mu) * rstd, (ld(D2) - mu) * rstd
        ops = _sb(t[:, :128], t[:, 128:], b[:, :128], b[:, 128:])
        for k in range(7):
            sb_s[zi, r0:r0 + 16, k * 128:(k + 1) * 128] = ops[k]
        x1_s[0, pl.ds(pl.multiple_of(zi * 16 + D + (r0 % 32) // 2, 8), 8), 0:128] = t[:8, :128] + b[:8, 128:]

    grow = jax.lax.broadcasted_iota(jnp.int32, (GR, TQ), 0)
    sbuf = (sA, sB)
    qm, pmax, mx, acc = [None] * NP, [None] * NP, [None] * NP, [None] * H

    def qk(p, c):
        g = p // 2
        if c == 0:
            qg = q_s[g * GR:(g + 1) * GR, :]
            z = jnp.zeros_like(qg)
            j = (2 * p) % 4
            qm[p] = jnp.concatenate(
                [jnp.where((grow >= jj * DH) & (grow < (jj + 1) * DH), qg, z) for jj in (j, j + 1)], axis=1)
        s = _dot(k_s[g, c * KC:(c + 1) * KC, :], qm[p])
        sbuf[p % 2][zi, c * KC:(c + 1) * KC, :] = s
        pm = jnp.max(s.reshape(KC // 8, 8, 2 * TQ), axis=0)
        pmax[p] = pm if c == 0 else jnp.maximum(pmax[p], pm)
        if c == NK - 1:
            mx[p] = jnp.max(pmax[p], axis=0, keepdims=True)

    def sm(p, c):
        e, cc = c % 2, c // 2
        h = 2 * p + e
        rows = slice(cc * 2 * KC, (cc + 1) * 2 * KC)
        pp = jnp.exp2(sbuf[p % 2][zi, rows, e * TQ:(e + 1) * TQ] - mx[p][:, e * TQ:(e + 1) * TQ]).astype(bf16)
        d = _dot(vT_s[h * HP:(h + 1) * HP, rows], pp)
        acc[h] = d if cc == 0 else acc[h] + d
        if cc == NK // 2 - 1:
            oT_s[h * HP:(h + 1) * HP, :] = acc[h] * (1.0 / acc[h][DH:DH + 1, :])

    um = [[None] * 7 for _ in range(NC)]
    tb, dm, last, ob = [None] * NC, [None] * 7, [None] * 7, []
    hg = 0.5 * (1.0 - gt)
    hq = (hg[:, :128], hg[:, 128:]) * 2

    def up(c, k):
        um[c][k] = _dot(s3_s[k, c * 128:(c + 1) * 128, :], sb_s[zi, :, k * 128:(k + 1) * 128])
        if k == 5:
            tb[c] = _sb(*[_gelu(t, hh) for t, hh in zip(_sc(um[c]), hq)])

    def down(c, k):
        rb, cb = SDPOS[k]
        d = _dot(w4_s[rb:rb + D2, cb + c * 128:cb + (c + 1) * 128], tb[c][k])
        if c == NC - 1 and k in (1, 2, 5, 6):
            last[k] = d
        else:
            dm[k] = d if c == 0 else dm[k] + d

    def oproj(_, k):
        if not ob:
            ob.extend(_sb(*_quad(oT_s[...] * gt)))
        dm[k] = dm[k] + _dot(so_s[k], ob[k])

    dots = []
    for c in range(NC):
        dots += [(up, c, k) for k in (0, 3, 4, 6, 2, 1, 5)]
        if c >= 1:
            dots += [(down, c - 1, k) for k in range(7)]
    dots += [(oproj, 0, k) for k in range(7)]
    dots += [(down, NC - 1, k) for k in (0, 3, 4, 1, 2, 5, 6)]

    for n in range(NP * NK):
        qk(n // NK, n % NK)
        if n >= NK:
            sm(n // NK - 1, n % NK)
    for n, (fn, c, k) in enumerate(dots):
        fn(c, k)
        if n % 3 == 2 and n // 3 < NK:
            sm(NP - 1, n // 3)

    base = [xg + cc for xg, cc in zip(_quad(x1_s[zi, 0:D, :] * (1.0 - gt)), _sc(dm))]
    top = jnp.concatenate([base[0] + last[6], base[1] + last[2]], axis=1).astype(bf16)
    bot = jnp.concatenate([base[2] + last[1], base[3] - last[1] + last[2] + last[5]], axis=1).astype(bf16)
    col0 = pl.multiple_of(i * TQ, TQ)
    for n, buf in enumerate((oa_s, ob_s)):
        buf[i, 0] = top[n * C:(n + 1) * C]
        buf[i, 1] = bot[n * C:(n + 1) * C]
        for e in range(2):
            cp(buf.at[i, e], o_hbm.at[pl.ds(e * D2 + n * C, C), pl.ds(col0, TQ)], osems.at[n]).start()

    @pl.when(i == NB - 1)
    def _drain():
        for n, buf in enumerate((oa_s, ob_s)):
            cp(buf, buf, osems.at[n]).wait()


@jax.jit
def pallas_gated_mix__mha_block__mixer_s_mlp__prompt_kernel(
    A_x: jax.Array,
    A_wqkv: jax.Array,
    A_wo: jax.Array,
    B_x: jax.Array,
    B_w1: jax.Array,
    B_w2: jax.Array,
    B_w3: jax.Array,
    B_w4: jax.Array,
    gate_w: jax.Array,
):
    args = (A_x.reshape(S, D).T, A_wqkv, A_wo, B_w1, B_w2, B_w3, B_w4.T, gate_w)
    out_t = pl.pallas_call(
        _kernel,
        grid=(NB,),
        in_specs=[pl.BlockSpec(memory_space=pl.ANY)] * len(args),
        out_specs=pl.BlockSpec(memory_space=pl.ANY),
        out_shape=jax.ShapeDtypeStruct((D, S), bf16),
        scratch_shapes=[pltpu.VMEM(*v) for v in SCRATCH.values()]
        + [pltpu.SemaphoreType.DMA((len(PLAN),)), pltpu.SemaphoreType.DMA((2,))],
        compiler_params=pltpu.CompilerParams(
            dimension_semantics=("arbitrary",), vmem_limit_bytes=100 * 1024 * 1024,
            disable_bounds_checks=True),
    )(*args)
    return out_t.T.reshape(1, S, D)
```

```python
import functools
import math

import jax
import jax.numpy as jnp
import jax.experimental.pallas as pl
import jax.experimental.pallas.tpu as pltpu

S, D, H, DH, F = 2048, 448, 16, 28, 1792
HP = 32
DP = H * HP
GR = 4 * DH
TQ = 256
NB = S // TQ
KC = 128
NK = S // KC
NP = H // 2
FH, D2, DP2 = F // 2, D // 2, DP // 2
NC = FH // 128
C = D // 4
HALO = 128
EPS = 1e-5
QSCALE = (DH ** -0.5) * math.log2(math.e)
f32, bf16 = jnp.float32, jnp.bfloat16

SDPOS = {2: (0, 0), 3: (D2, FH), 0: (D, 0), 1: (D, FH), 4: (D + D2, 0), 5: (D + D2, FH), 6: (2 * D, 0)}
PLAN = [
    ("g wka", "Twka Tg"),
    ("x0", "Ka0 S0"),
    ("wkb", "Twkb Kb0"),
    ("x1 x2", "K1 S1 K2 S2"),
    ("x3 x4 x5 x6", "K3 S3 T0 K4 S4 T1 K5 S5 S6"),
    ("x7 w1 wv wq", "Tw1 K6 K7 S7 Twv Twq W0 T2 W7 T3 W1 T4 W2 T5 W3 T6 W4 T7 W5 W6"),
    ("w2 wo w3 w4", "Tw2 Two Tw3 Tw4 V0 H0 V1 H1 V2 H2 V3 H3 V4 H4 V5 H5 V6 H6 V7 H7"),
]
SCRATCH = dict(
    gw_r=((D,), bf16),
    sA=((1, S, 2 * TQ), f32), sB=((1, S, 2 * TQ), f32), k_s=((4, S, GR), bf16), vT_s=((DP, S), bf16),
    x_s=((NB, D, TQ), bf16), wqkv_r=((D, 3 * D), bf16), wo_r=((D, D), bf16), w1_r=((D, D), bf16),
    w2_r=((D, D), bf16), w3_r=((D, F), bf16), w4_s=((D + 3 * D2, F), bf16),
    wqkvT_s=((3 * D, D), bf16), so_s=((7, D2, DP2), bf16), w1T_s=((D, D), bf16),
    s2_s=((7, D2, D2), bf16), s3_s=((7, FH, D2), bf16), wop_s=((DP, D), f32),
    kT_s=((NB, D, TQ), bf16), st_s=((NB, 8, TQ), f32),
    h_s=((D, S + 2 * HALO), bf16), hs_s=((NB, D, TQ), bf16), q_s=((D, TQ), bf16), oT_s=((DP, TQ), f32),
    oa_s=((NB, 2, C, TQ), bf16), ob_s=((NB, 2, C, TQ), bf16), x1_s=((1, D + 16, TQ), f32),
    sb_s=((1, D2, 7 * 128), bf16), gcol_s=((D + 8, 128), f32), scol_s=((D, 128), f32))


def _gelu(x, half=0.5):
    c = math.sqrt(2.0 / math.pi)
    return half * x * (1.0 + jnp.tanh(c * (x + 0.044715 * (x * x * x))))


def _dot(a, b):
    return jnp.dot(a, b, preferred_element_type=f32)


def _ln_stats(x):
    c0 = x[0:1, :]
    d = x - c0
    m1 = jnp.mean(d, axis=0, keepdims=True)
    m2 = jnp.mean(d * d, axis=0, keepdims=True)
    return c0 + m1, jax.lax.rsqrt(jnp.maximum(m2 - m1 * m1, 0.0) + EPS)


def _sa(a11, a12, a21, a22):
    return [a11 + a22, a21 + a22, a11, a22, a11 + a12, a21 - a11, a12 - a22]


def _sb(b11, b12, b21, b22):
    return [t.astype(bf16) for t in (b11 + b22, b11, b12 - b22, b21 - b11, b22, b11 + b12, b21 + b22)]


def _sc(m):
    return m[0] + m[3] - m[4] + m[6], m[2] + m[4], m[1] + m[3], m[0] - m[1] + m[2] + m[5]


def _quad(x):
    r = x.shape[0] // 2
    return x[:r, :128], x[:r, 128:], x[r:, :128], x[r:, 128:]


def _col(row):
    return jnp.broadcast_to(row, (128, D)).T


def _wide(col):
    return jnp.concatenate([col] * (TQ // 128), axis=1)


def _kernel(x_hbm, wqkv_hbm, wo_hbm, w1_hbm, w2_hbm, w3_hbm, w4T_hbm, gw_hbm, o_hbm,
            gw_r, sA, sB, k_s, vT_s, x_s, wqkv_r, wo_r, w1_r, w2_r, w3_r, w4_s, wqkvT_s, so_s, w1T_s,
            s2_s, s3_s, wop_s, kT_s, st_s, h_s, hs_s, q_s, oT_s, oa_s, ob_s, x1_s, sb_s, gcol_s, scol_s,
            sems, osems):
    i = pl.program_id(0)
    zi = jnp.minimum(i, 0)
    cp = pltpu.make_async_copy

    @pl.when(i == 0)
    def _prologue():
        row = jax.lax.broadcasted_iota(jnp.int32, (HP - DH, TQ), 0)
        pad_rows = jnp.where(row == 0, 1.0, 0.0)

        tick = []

        def kproj(b, lo=0, hi=D):
            kT_s[b, lo:hi, :] = _dot(wqkvT_s[D + lo:D + hi, :], x_s[b]).astype(bf16)

        def ktr(b):
            for g in range(4):
                k_s[g, b * TQ:(b + 1) * TQ, :] = kT_s[b, g * GR:(g + 1) * GR, :].T

        def stats(b):
            if b == NB - 1:
                xf = x_s[b].astype(f32)
                mu, rstd = _ln_stats(xf)
                z = jnp.sum(xf * _wide(gcol_s[0:D, :]), axis=0, keepdims=True)
            else:
                c0 = x_s[b, 0:16, :].astype(f32)[0:1, :]
                if not tick:
                    tick.append(jnp.where(i < 0, jnp.broadcast_to(c0[:, :128], (8, 128)), 0.0))
                tot = None
                for r0 in range(0, D, 16):
                    tick[0] = jnp.tanh(jnp.tanh(jnp.tanh(tick[0])))
                    c8 = c0 + jnp.concatenate([tick[0], tick[0]], axis=1)
                    d = x_s[b, r0:r0 + 16, :].astype(f32) - jnp.concatenate([c8, c8], axis=0)
                    part = [t[:8] + t[8:] for t in (d, d * d, d * _wide(gcol_s[r0:r0 + 16, :]))]
                    tot = part if tot is None else [s + t for s, t in zip(tot, part)]
                s1, s2, s3 = [jnp.sum(t, axis=0, keepdims=True) for t in tot]
                m1, m2 = s1 * (1.0 / D), s2 * (1.0 / D)
                mu = c0 + m1
                rstd = jax.lax.rsqrt(jnp.maximum(m2 - m1 * m1, 0.0) + EPS)
                z = s3 + c0 * _wide(gcol_s[D:D + 1, :])
            st_s[b, 0:1, :] = rstd
            st_s[b, 1:2, :] = mu * rstd
            st_s[b, 2:3, :] = jax.nn.sigmoid(z)

        def w1proj(b):
            y = _dot(w1T_s[...], x_s[b])
            pre = y * st_s[b, 0:1, :] - _wide(scol_s[...]) * st_s[b, 1:2, :]
            h_s[:, HALO + b * TQ:HALO + (b + 1) * TQ] = _gelu(pre).astype(bf16)

        def vproj(b):
            v = _dot(wqkvT_s[2 * D:, :], x_s[b])
            for h in range(H):
                vT_s[h * HP:(h + 1) * HP, b * TQ:(b + 1) * TQ] = jnp.concatenate(
                    [v[h * DH:(h + 1) * DH, :], pad_rows], axis=0).astype(bf16)

        def shift(b):
            l0 = HALO + b * TQ
            for g, off in enumerate((-1, 1, -2, 2)):
                hs_s[b, g * C:(g + 1) * C, :] = h_s[g * C:(g + 1) * C, l0 + off:l0 + off + TQ]

        def t_qkv(lo, hi):
            wqkvT_s[lo:hi, :] = wqkv_r[:, lo:hi].T

        def t_w1():
            w1T_s[...] = w1_r[...].T
            scol_s[...] = _col(jnp.sum(w1_r[...].astype(f32), axis=0, keepdims=True))

        def left_ops(w, dst):
            kh = w.shape[0] // 2
            t1, t2 = w[:kh].T.astype(f32), w[kh:].T.astype(f32)
            for k, a in enumerate(_sa(t1[:D2], t2[:D2], t1[D2:], t2[D2:])):
                dst[k] = a.astype(bf16)

        def t_wo():
            wof = wo_r[...].astype(f32)
            for h in range(H):
                wop_s[h * HP:h * HP + DH, :] = wof[h * DH:(h + 1) * DH, :]
            left_ops(wop_s[...].astype(bf16), so_s)

        def t_w3():
            for c in range(NC):
                def blk(r, e):
                    return w3_r[r * D2:(r + 1) * D2, e * FH + c * 128:e * FH + (c + 1) * 128].astype(f32)
                for k, a in enumerate(_sa(blk(0, 0), blk(1, 0), blk(0, 1), blk(1, 1))):
                    s3_s[k, c * 128:(c + 1) * 128, :] = a.astype(bf16).T

        def t_w4():
            for r0 in range(0, D2, 16):
                def rows(base):
                    return pl.ds(pl.multiple_of(zi * 16 + base + r0, 16), 16)
                for c0 in range(0, FH, 256):
                    c1 = min(c0 + 256, FH)
                    def blk(r, e):
                        return w4_s[rows(r * D2), e * FH + c0:e * FH + c1].astype(f32)
                    for k, a in enumerate(_sa(blk(0, 0), blk(0, 1), blk(1, 0), blk(1, 1))):
                        if k not in (2, 3):
                            rb, cb = SDPOS[k]
                            w4_s[rows(rb), cb + c0:cb + c1] = a.astype(bf16)

        def t_g():
            gc = _col(gw_r[...].astype(f32).reshape(1, D))
            gcol_s[0:D, :] = gc
            gcol_s[D:D + 1, :] = jnp.sum(gc, axis=0, keepdims=True)

        def cols(lo, n):
            return wqkv_hbm.at[:, pl.ds(lo, n)], wqkv_r.at[:, pl.ds(lo, n)]

        copies = {"g": (gw_hbm, gw_r), "wka": cols(640, 256), "wkb": cols(384, 256),
                  "wv": cols(896, 448), "wq": cols(0, 384),
                  "w1": (w1_hbm, w1_r), "w2": (w2_hbm, w2_r), "wo": (wo_hbm, wo_r), "w3": (w3_hbm, w3_r),
                  "w4": (w4T_hbm, w4_s.at[pl.ds(0, D), :])}
        jobs = {"Twka": functools.partial(t_qkv, 640, 896), "Twkb": functools.partial(t_qkv, 384, 640),
                "Twv": functools.partial(t_qkv, 896, 3 * D), "Twq": functools.partial(t_qkv, 0, 384),
                "Ka0": functools.partial(kproj, 0, 640 - D, D), "Kb0": functools.partial(kproj, 0, 0, 640 - D),
                "Tw1": t_w1,
                "Tw2": lambda: left_ops(w2_r[...], s2_s), "Two": t_wo, "Tw3": t_w3, "Tw4": t_w4, "Tg": t_g}
        for b in range(NB):
            copies["x%d" % b] = (x_hbm.at[:, pl.ds(b * TQ, TQ)], x_s.at[b])
            for nm, fn in (("K", kproj), ("T", ktr), ("S", stats), ("W", w1proj), ("V", vproj), ("H", shift)):
                jobs["%s%d" % (nm, b)] = functools.partial(fn, b)

        grp = [[cp(*copies[n], sems.at[k]) for n in g.split()] for k, (g, _) in enumerate(PLAN)]
        for g in grp:
            for c in g:
                c.start()
        h_s[:, 0:HALO] = jnp.zeros((D, HALO), bf16)
        h_s[:, HALO + S:] = jnp.zeros((D, HALO), bf16)
        wop_s[...] = jnp.zeros(wop_s.shape, f32)
        for k, (_, js) in enumerate(PLAN):
            for c in grp[k]:
                c.wait()
            tick.clear()
            for j in js.split():
                jobs[j]()

    xb = x_s[i]
    q_s[...] = (_dot(wqkvT_s[0:D, :], xb) * QSCALE).astype(bf16)
    gt = st_s[i, 2:3, :]

    hb = _sb(*_quad(hs_s[i].astype(f32)))
    c11, c12, c21, c22 = _sc([_dot(s2_s[k], hb[k]) for k in range(7)])
    x1 = xb.astype(f32) + jnp.concatenate(
        [jnp.concatenate([c11, c12], axis=1), jnp.concatenate([c21, c22], axis=1)], axis=0)
    x1_s[zi, 0:D, :] = x1
    mu, rstd = _ln_stats(x1)
    mu = jnp.broadcast_to(mu, (16, TQ))
    rstd = jnp.broadcast_to(rstd, (16, TQ))
    for r0 in range(0, D2, 16):
        def ld(base):
            return x1_s[0, pl.ds(pl.multiple_of(zi * 16 + base + r0, 16), 16), :]
        t, b = (ld(0) - mu) * rstd, (ld(D2) - mu) * rstd
        ops = _sb(t[:, :128], t[:, 128:], b[:, :128], b[:, 128:])
        for k in range(7):
            sb_s[zi, r0:r0 + 16, k * 128:(k + 1) * 128] = ops[k]
        x1_s[0, pl.ds(pl.multiple_of(zi * 16 + D + (r0 % 32) // 2, 8), 8), 0:128] = t[:8, :128] + b[:8, 128:]

    grow = jax.lax.broadcasted_iota(jnp.int32, (GR, TQ), 0)
    sbuf = (sA, sB)
    qm, pmax, mx, acc = [None] * NP, [None] * NP, [None] * NP, [None] * H

    def qk(p, c):
        g = p // 2
        if c == 0:
            qg = q_s[g * GR:(g + 1) * GR, :]
            z = jnp.zeros_like(qg)
            j = (2 * p) % 4
            qm[p] = jnp.concatenate(
                [jnp.where((grow >= jj * DH) & (grow < (jj + 1) * DH), qg, z) for jj in (j, j + 1)], axis=1)
        s = _dot(k_s[g, c * KC:(c + 1) * KC, :], qm[p])
        sbuf[p % 2][zi, c * KC:(c + 1) * KC, :] = s
        pm = jnp.max(s.reshape(KC // 8, 8, 2 * TQ), axis=0)
        pmax[p] = pm if c == 0 else jnp.maximum(pmax[p], pm)
        if c == NK - 1:
            mx[p] = jnp.max(pmax[p], axis=0, keepdims=True)

    def sm(p, c):
        e, cc = c % 2, c // 2
        h = 2 * p + e
        rows = slice(cc * 2 * KC, (cc + 1) * 2 * KC)
        pp = jnp.exp2(sbuf[p % 2][zi, rows, e * TQ:(e + 1) * TQ] - mx[p][:, e * TQ:(e + 1) * TQ]).astype(bf16)
        d = _dot(vT_s[h * HP:(h + 1) * HP, rows], pp)
        acc[h] = d if cc == 0 else acc[h] + d
        if cc == NK // 2 - 1:
            oT_s[h * HP:(h + 1) * HP, :] = acc[h] * (1.0 / acc[h][DH:DH + 1, :])

    um = [[None] * 7 for _ in range(NC)]
    tb, dm, last, ob = [None] * NC, [None] * 7, [None] * 7, []
    hg = 0.5 * (1.0 - gt)
    hq = (hg[:, :128], hg[:, 128:]) * 2

    def up(c, k):
        um[c][k] = _dot(s3_s[k, c * 128:(c + 1) * 128, :], sb_s[zi, :, k * 128:(k + 1) * 128])
        if k == 5:
            tb[c] = _sb(*[_gelu(t, hh) for t, hh in zip(_sc(um[c]), hq)])

    def down(c, k):
        rb, cb = SDPOS[k]
        d = _dot(w4_s[rb:rb + D2, cb + c * 128:cb + (c + 1) * 128], tb[c][k])
        if c == NC - 1 and k in (1, 2, 5, 6):
            last[k] = d
        else:
            dm[k] = d if c == 0 else dm[k] + d

    def oproj(_, k):
        if not ob:
            ob.extend(_sb(*_quad(oT_s[...] * gt)))
        dm[k] = dm[k] + _dot(so_s[k], ob[k])

    dots = []
    for c in range(NC):
        dots += [(up, c, k) for k in (0, 3, 4, 6, 2, 1, 5)]
        if c >= 1:
            dots += [(down, c - 1, k) for k in range(7)]
    dots += [(oproj, 0, k) for k in range(7)]
    dots += [(down, NC - 1, k) for k in (0, 3, 4, 1, 2, 5, 6)]

    for n in range(NP * NK):
        qk(n // NK, n % NK)
        if n >= NK:
            sm(n // NK - 1, n % NK)
    for n, (fn, c, k) in enumerate(dots):
        fn(c, k)
        if n % 3 == 2 and n // 3 < NK:
            sm(NP - 1, n // 3)

    base = [xg + cc for xg, cc in zip(_quad(x1_s[zi, 0:D, :] * (1.0 - gt)), _sc(dm))]
    top = jnp.concatenate([base[0] + last[6], base[1] + last[2]], axis=1).astype(bf16)
    bot = jnp.concatenate([base[2] + last[1], base[3] - last[1] + last[2] + last[5]], axis=1).astype(bf16)
    col0 = pl.multiple_of(i * TQ, TQ)
    for n, buf in enumerate((oa_s, ob_s)):
        buf[i, 0] = top[n * C:(n + 1) * C]
        buf[i, 1] = bot[n * C:(n + 1) * C]
        for e in range(2):
            cp(buf.at[i, e], o_hbm.at[pl.ds(e * D2 + n * C, C), pl.ds(col0, TQ)], osems.at[n]).start()

    @pl.when(i == NB - 1)
    def _drain():
        for n, buf in enumerate((oa_s, ob_s)):
            cp(buf, buf, osems.at[n]).wait()


@jax.jit
def pallas_gated_mix__mha_block__mixer_s_mlp__prompt_kernel(
    A_x: jax.Array,
    A_wqkv: jax.Array,
    A_wo: jax.Array,
    B_x: jax.Array,
    B_w1: jax.Array,
    B_w2: jax.Array,
    B_w3: jax.Array,
    B_w4: jax.Array,
    gate_w: jax.Array,
):
    args = (A_x.reshape(S, D).T, A_wqkv, A_wo, B_w1, B_w2, B_w3, B_w4.T, gate_w)
    out_t = pl.pallas_call(
        _kernel,
        grid=(NB,),
        in_specs=[pl.BlockSpec(memory_space=pl.ANY)] * len(args),
        out_specs=pl.BlockSpec(memory_space=pl.ANY),
        out_shape=jax.ShapeDtypeStruct((D, S), bf16),
        scratch_shapes=[pltpu.VMEM(*v) for v in SCRATCH.values()]
        + [pltpu.SemaphoreType.DMA((len(PLAN),)), pltpu.SemaphoreType.DMA((2,))],
        compiler_params=pltpu.CompilerParams(
            dimension_semantics=("arbitrary",), vmem_limit_bytes=100 * 1024 * 1024,
            disable_bounds_checks=True),
    )(*args)
    return out_t.T.reshape(1, S, D)
```

```python
import functools
import math

import jax
import jax.numpy as jnp
import jax.experimental.pallas as pl
import jax.experimental.pallas.tpu as pltpu

S, D, H, DH, F = 2048, 448, 16, 28, 1792
HP = 32
DP = H * HP
GR = 4 * DH
TQ = 256
NB = S // TQ
KC = 128
NK = S // KC
NP = H // 2
FH, D2 = F // 2, D // 2
NC = FH // 128
C = D // 4
HALO = 128
EPS = 1e-5
QSCALE = (DH ** -0.5) * math.log2(math.e)
f32, bf16 = jnp.float32, jnp.bfloat16

SDPOS = {2: (0, 0), 3: (D2, FH), 0: (D, 0), 1: (D, FH), 4: (D + D2, 0), 5: (D + D2, FH), 6: (2 * D, 0)}
PLAN = [
    ("g wka", "Twka Tg"),
    ("x0", "Ka0 S0"),
    ("wkb", "Twkb Kb0"),
    ("x1 x2", "K1 S1 K2 S2"),
    ("x3 x4 x5 x6", "K3 S3 T0 K4 S4 T1 K5 S5 S6"),
    ("x7 w1 wv wq", "Tw1 K6 K7 S7 Twv Twq W0 T2 W7 T3 W1 T4 W2 T5 W3 T6 W4 T7 W5 W6"),
    ("w2 wo w3 w4", "Tw2 Two Tw3 Tw4 V0 H0 V1 H1 V2 H2 V3 H3 V4 H4 V5 H5 V6 H6 V7 H7"),
]
SCRATCH = dict(
    gw_r=((D,), bf16),
    sA=((1, S, 2 * TQ), f32), sB=((1, S, 2 * TQ), f32), k_s=((4, S, GR), bf16), vT_s=((DP, S), bf16),
    x_s=((NB, D, TQ), bf16), wqkv_r=((D, 3 * D), bf16), wo_r=((D, D), bf16), w1_r=((D, D), bf16),
    w2_r=((D, D), bf16), w3_r=((D, F), bf16), w4_s=((D + 3 * D2, F), bf16),
    wqkvT_s=((3 * D, D), bf16), so_s=((7, D2, D2), bf16), w1T_s=((D, D), bf16),
    s2_s=((7, D2, D2), bf16), s3_s=((7, FH, D2), bf16),
    kT_s=((NB, D, TQ), bf16), st_s=((NB, 8, TQ), f32),
    h_s=((D, S + 2 * HALO), bf16), hs_s=((NB, D, TQ), bf16), q_s=((D, TQ), bf16),
    oa_s=((NB, 2, C, TQ), bf16), ob_s=((NB, 2, C, TQ), bf16), x1_s=((1, D + 16, TQ), f32),
    sb_s=((1, D2, 7 * 128), bf16), gcol_s=((D + 8, 128), f32), scol_s=((D, 128), f32))


def _gelu(x, half=0.5):
    c = math.sqrt(2.0 / math.pi)
    return half * x * (1.0 + jnp.tanh(c * (x + 0.044715 * (x * x * x))))


def _dot(a, b):
    return jnp.dot(a, b, preferred_element_type=f32)


def _ln_stats(x):
    c0 = x[0:1, :]
    d = x - c0
    m1 = jnp.mean(d, axis=0, keepdims=True)
    m2 = jnp.mean(d * d, axis=0, keepdims=True)
    return c0 + m1, jax.lax.rsqrt(jnp.maximum(m2 - m1 * m1, 0.0) + EPS)


def _sa(a11, a12, a21, a22):
    return [a11 + a22, a21 + a22, a11, a22, a11 + a12, a21 - a11, a12 - a22]


def _sb(b11, b12, b21, b22):
    return [t.astype(bf16) for t in (b11 + b22, b11, b12 - b22, b21 - b11, b22, b11 + b12, b21 + b22)]


def _sc(m):
    return m[0] + m[3] - m[4] + m[6], m[2] + m[4], m[1] + m[3], m[0] - m[1] + m[2] + m[5]


def _quad(x):
    r = x.shape[0] // 2
    return x[:r, :128], x[:r, 128:], x[r:, :128], x[r:, 128:]


def _col(row):
    return jnp.broadcast_to(row, (128, D)).T


def _wide(col):
    return jnp.concatenate([col] * (TQ // 128), axis=1)


def _kernel(x_hbm, wqkv_hbm, wo_hbm, w1_hbm, w2_hbm, w3_hbm, w4T_hbm, gw_hbm, o_hbm,
            gw_r, sA, sB, k_s, vT_s, x_s, wqkv_r, wo_r, w1_r, w2_r, w3_r, w4_s, wqkvT_s, so_s, w1T_s,
            s2_s, s3_s, kT_s, st_s, h_s, hs_s, q_s, oa_s, ob_s, x1_s, sb_s, gcol_s, scol_s,
            sems, osems):
    i = pl.program_id(0)
    zi = jnp.minimum(i, 0)
    cp = pltpu.make_async_copy

    @pl.when(i == 0)
    def _prologue():
        row = jax.lax.broadcasted_iota(jnp.int32, (HP - DH, TQ), 0)
        pad_rows = jnp.where(row == 0, 1.0, 0.0)

        tick = []

        def kproj(b, lo=0, hi=D):
            kT_s[b, lo:hi, :] = _dot(wqkvT_s[D + lo:D + hi, :], x_s[b]).astype(bf16)

        def ktr(b):
            for g in range(4):
                k_s[g, b * TQ:(b + 1) * TQ, :] = kT_s[b, g * GR:(g + 1) * GR, :].T

        def stats(b):
            if b == NB - 1:
                xf = x_s[b].astype(f32)
                mu, rstd = _ln_stats(xf)
                z = jnp.sum(xf * _wide(gcol_s[0:D, :]), axis=0, keepdims=True)
            else:
                c0 = x_s[b, 0:16, :].astype(f32)[0:1, :]
                if not tick:
                    tick.append(jnp.where(i < 0, jnp.broadcast_to(c0[:, :128], (8, 128)), 0.0))
                tot = None
                for r0 in range(0, D, 16):
                    tick[0] = jnp.tanh(jnp.tanh(jnp.tanh(tick[0])))
                    c8 = c0 + jnp.concatenate([tick[0], tick[0]], axis=1)
                    d = x_s[b, r0:r0 + 16, :].astype(f32) - jnp.concatenate([c8, c8], axis=0)
                    part = [t[:8] + t[8:] for t in (d, d * d, d * _wide(gcol_s[r0:r0 + 16, :]))]
                    tot = part if tot is None else [s + t for s, t in zip(tot, part)]
                s1, s2, s3 = [jnp.sum(t, axis=0, keepdims=True) for t in tot]
                m1, m2 = s1 * (1.0 / D), s2 * (1.0 / D)
                mu = c0 + m1
                rstd = jax.lax.rsqrt(jnp.maximum(m2 - m1 * m1, 0.0) + EPS)
                z = s3 + c0 * _wide(gcol_s[D:D + 1, :])
            st_s[b, 0:1, :] = rstd
            st_s[b, 1:2, :] = mu * rstd
            st_s[b, 2:3, :] = jax.nn.sigmoid(z)

        def w1proj(b):
            y = _dot(w1T_s[...], x_s[b])
            pre = y * st_s[b, 0:1, :] - _wide(scol_s[...]) * st_s[b, 1:2, :]
            h_s[:, HALO + b * TQ:HALO + (b + 1) * TQ] = _gelu(pre).astype(bf16)

        def vproj(b):
            v = _dot(wqkvT_s[2 * D:, :], x_s[b])
            for h in range(H):
                vT_s[h * HP:(h + 1) * HP, b * TQ:(b + 1) * TQ] = jnp.concatenate(
                    [v[h * DH:(h + 1) * DH, :], pad_rows], axis=0).astype(bf16)

        def shift(b):
            l0 = HALO + b * TQ
            for g, off in enumerate((-1, 1, -2, 2)):
                hs_s[b, g * C:(g + 1) * C, :] = h_s[g * C:(g + 1) * C, l0 + off:l0 + off + TQ]

        def t_qkv(lo, hi):
            wqkvT_s[lo:hi, :] = wqkv_r[:, lo:hi].T

        def t_w1():
            w1T_s[...] = w1_r[...].T
            scol_s[...] = _col(jnp.sum(w1_r[...].astype(f32), axis=0, keepdims=True))

        def left_ops(w, dst):
            t1, t2 = w[:D2].T.astype(f32), w[D2:].T.astype(f32)
            for k, a in enumerate(_sa(t1[:D2], t2[:D2], t1[D2:], t2[D2:])):
                dst[k] = a.astype(bf16)

        def t_w3():
            for c in range(NC):
                def blk(r, e):
                    return w3_r[r * D2:(r + 1) * D2, e * FH + c * 128:e * FH + (c + 1) * 128].astype(f32)
                for k, a in enumerate(_sa(blk(0, 0), blk(1, 0), blk(0, 1), blk(1, 1))):
                    s3_s[k, c * 128:(c + 1) * 128, :] = a.astype(bf16).T

        def t_w4():
            for r0 in range(0, D2, 16):
                def rows(base):
                    return pl.ds(pl.multiple_of(zi * 16 + base + r0, 16), 16)
                for c0 in range(0, FH, 256):
                    c1 = min(c0 + 256, FH)
                    def blk(r, e):
                        return w4_s[rows(r * D2), e * FH + c0:e * FH + c1].astype(f32)
                    for k, a in enumerate(_sa(blk(0, 0), blk(0, 1), blk(1, 0), blk(1, 1))):
                        if k not in (2, 3):
                            rb, cb = SDPOS[k]
                            w4_s[rows(rb), cb + c0:cb + c1] = a.astype(bf16)

        def t_g():
            gc = _col(gw_r[...].astype(f32).reshape(1, D))
            gcol_s[0:D, :] = gc
            gcol_s[D:D + 1, :] = jnp.sum(gc, axis=0, keepdims=True)

        def cols(lo, n):
            return wqkv_hbm.at[:, pl.ds(lo, n)], wqkv_r.at[:, pl.ds(lo, n)]

        copies = {"g": (gw_hbm, gw_r), "wka": cols(640, 256), "wkb": cols(384, 256),
                  "wv": cols(896, 448), "wq": cols(0, 384),
                  "w1": (w1_hbm, w1_r), "w2": (w2_hbm, w2_r), "wo": (wo_hbm, wo_r), "w3": (w3_hbm, w3_r),
                  "w4": (w4T_hbm, w4_s.at[pl.ds(0, D), :])}
        jobs = {"Twka": functools.partial(t_qkv, 640, 896), "Twkb": functools.partial(t_qkv, 384, 640),
                "Twv": functools.partial(t_qkv, 896, 3 * D), "Twq": functools.partial(t_qkv, 0, 384),
                "Ka0": functools.partial(kproj, 0, 640 - D, D), "Kb0": functools.partial(kproj, 0, 0, 640 - D),
                "Tw1": t_w1,
                "Tw2": lambda: left_ops(w2_r[...], s2_s), "Two": lambda: left_ops(wo_r[...], so_s),
                "Tw3": t_w3, "Tw4": t_w4, "Tg": t_g}
        for b in range(NB):
            copies["x%d" % b] = (x_hbm.at[:, pl.ds(b * TQ, TQ)], x_s.at[b])
            for nm, fn in (("K", kproj), ("T", ktr), ("S", stats), ("W", w1proj), ("V", vproj), ("H", shift)):
                jobs["%s%d" % (nm, b)] = functools.partial(fn, b)

        grp = [[cp(*copies[n], sems.at[k]) for n in g.split()] for k, (g, _) in enumerate(PLAN)]
        for g in grp:
            for c in g:
                c.start()
        h_s[:, 0:HALO] = jnp.zeros((D, HALO), bf16)
        h_s[:, HALO + S:] = jnp.zeros((D, HALO), bf16)
        for k, (_, js) in enumerate(PLAN):
            for c in grp[k]:
                c.wait()
            tick.clear()
            for j in js.split():
                jobs[j]()

    xb = x_s[i]
    q_s[...] = (_dot(wqkvT_s[0:D, :], xb) * QSCALE).astype(bf16)
    gt = st_s[i, 2:3, :]

    hb = _sb(*_quad(hs_s[i].astype(f32)))
    c11, c12, c21, c22 = _sc([_dot(s2_s[k], hb[k]) for k in range(7)])
    x1 = xb.astype(f32) + jnp.concatenate(
        [jnp.concatenate([c11, c12], axis=1), jnp.concatenate([c21, c22], axis=1)], axis=0)
    x1_s[zi, 0:D, :] = x1
    mu, rstd = _ln_stats(x1)
    mu = jnp.broadcast_to(mu, (16, TQ))
    rstd = jnp.broadcast_to(rstd, (16, TQ))
    for r0 in range(0, D2, 16):
        def ld(base):
            return x1_s[0, pl.ds(pl.multiple_of(zi * 16 + base + r0, 16), 16), :]
        t, b = (ld(0) - mu) * rstd, (ld(D2) - mu) * rstd
        ops = _sb(t[:, :128], t[:, 128:], b[:, :128], b[:, 128:])
        for k in range(7):
            sb_s[zi, r0:r0 + 16, k * 128:(k + 1) * 128] = ops[k]
        x1_s[0, pl.ds(pl.multiple_of(zi * 16 + D + (r0 % 32) // 2, 8), 8), 0:128] = t[:8, :128] + b[:8, 128:]

    grow = jax.lax.broadcasted_iota(jnp.int32, (GR, TQ), 0)
    sbuf = (sA, sB)
    qm, pmax, mx, acc = [None] * NP, [None] * NP, [None] * NP, [None] * H

    def qk(p, c):
        g = p // 2
        if c == 0:
            qg = q_s[g * GR:(g + 1) * GR, :]
            z = jnp.zeros_like(qg)
            j = (2 * p) % 4
            qm[p] = jnp.concatenate(
                [jnp.where((grow >= jj * DH) & (grow < (jj + 1) * DH), qg, z) for jj in (j, j + 1)], axis=1)
        s = _dot(k_s[g, c * KC:(c + 1) * KC, :], qm[p])
        sbuf[p % 2][zi, c * KC:(c + 1) * KC, :] = s
        pm = jnp.max(s.reshape(KC // 8, 8, 2 * TQ), axis=0)
        pmax[p] = pm if c == 0 else jnp.maximum(pmax[p], pm)
        if c == NK - 1:
            mx[p] = jnp.max(pmax[p], axis=0, keepdims=True)

    def sm(p, c):
        e, cc = c % 2, c // 2
        h = 2 * p + e
        rows = slice(cc * 2 * KC, (cc + 1) * 2 * KC)
        pp = jnp.exp2(sbuf[p % 2][zi, rows, e * TQ:(e + 1) * TQ] - mx[p][:, e * TQ:(e + 1) * TQ]).astype(bf16)
        d = _dot(vT_s[h * HP:(h + 1) * HP, rows], pp)
        acc[h] = d if cc == 0 else acc[h] + d
        if cc == NK // 2 - 1:
            acc[h] = (acc[h] * (1.0 / acc[h][DH:DH + 1, :]))[:DH]

    um = [[None] * 7 for _ in range(NC)]
    tb, dm, last, ob = [None] * NC, [None] * 7, [None] * 7, []
    hg = 0.5 * (1.0 - gt)
    hq = (hg[:, :128], hg[:, 128:]) * 2

    def up(c, k):
        um[c][k] = _dot(s3_s[k, c * 128:(c + 1) * 128, :], sb_s[zi, :, k * 128:(k + 1) * 128])
        if k == 5:
            tb[c] = _sb(*[_gelu(t, hh) for t, hh in zip(_sc(um[c]), hq)])

    def down(c, k):
        rb, cb = SDPOS[k]
        d = _dot(w4_s[rb:rb + D2, cb + c * 128:cb + (c + 1) * 128], tb[c][k])
        if c == NC - 1 and k in (1, 2, 5, 6):
            last[k] = d
        else:
            dm[k] = d if c == 0 else dm[k] + d

    def oproj(_, k):
        if not ob:
            ob.extend(_sb(*_quad(jnp.concatenate(acc, axis=0) * gt)))
        dm[k] = dm[k] + _dot(so_s[k], ob[k])

    dots = []
    for c in range(NC):
        dots += [(up, c, k) for k in (0, 3, 4, 6, 2, 1, 5)]
        if c >= 1:
            dots += [(down, c - 1, k) for k in range(7)]
    dots += [(oproj, 0, k) for k in range(7)]
    dots += [(down, NC - 1, k) for k in (0, 3, 4, 1, 2, 5, 6)]

    for n in range(NP * NK):
        qk(n // NK, n % NK)
        if n >= NK:
            sm(n // NK - 1, n % NK)
    for n, (fn, c, k) in enumerate(dots):
        fn(c, k)
        if n % 3 == 2 and n // 3 < NK:
            sm(NP - 1, n // 3)

    base = [xg + cc for xg, cc in zip(_quad(x1_s[zi, 0:D, :] * (1.0 - gt)), _sc(dm))]
    top = jnp.concatenate([base[0] + last[6], base[1] + last[2]], axis=1).astype(bf16)
    bot = jnp.concatenate([base[2] + last[1], base[3] - last[1] + last[2] + last[5]], axis=1).astype(bf16)
    col0 = pl.multiple_of(i * TQ, TQ)
    for n, buf in enumerate((oa_s, ob_s)):
        buf[i, 0] = top[n * C:(n + 1) * C]
        buf[i, 1] = bot[n * C:(n + 1) * C]
        for e in range(2):
            cp(buf.at[i, e], o_hbm.at[pl.ds(e * D2 + n * C, C), pl.ds(col0, TQ)], osems.at[n]).start()

    @pl.when(i == NB - 1)
    def _drain():
        for n, buf in enumerate((oa_s, ob_s)):
            cp(buf, buf, osems.at[n]).wait()


@jax.jit
def pallas_gated_mix__mha_block__mixer_s_mlp__prompt_kernel(
    A_x: jax.Array,
    A_wqkv: jax.Array,
    A_wo: jax.Array,
    B_x: jax.Array,
    B_w1: jax.Array,
    B_w2: jax.Array,
    B_w3: jax.Array,
    B_w4: jax.Array,
    gate_w: jax.Array,
):
    args = (A_x.reshape(S, D).T, A_wqkv, A_wo, B_w1, B_w2, B_w3, B_w4.T, gate_w)
    out_t = pl.pallas_call(
        _kernel,
        grid=(NB,),
        in_specs=[pl.BlockSpec(memory_space=pl.ANY)] * len(args),
        out_specs=pl.BlockSpec(memory_space=pl.ANY),
        out_shape=jax.ShapeDtypeStruct((D, S), bf16),
        scratch_shapes=[pltpu.VMEM(*v) for v in SCRATCH.values()]
        + [pltpu.SemaphoreType.DMA((len(PLAN),)), pltpu.SemaphoreType.DMA((2,))],
        compiler_params=pltpu.CompilerParams(
            dimension_semantics=("arbitrary",), vmem_limit_bytes=100 * 1024 * 1024,
            disable_bounds_checks=True),
    )(*args)
    return out_t.T.reshape(1, S, D)
```

```python
import functools
import math

import jax
import jax.numpy as jnp
import jax.experimental.pallas as pl
import jax.experimental.pallas.tpu as pltpu

S, D, H, DH, F = 2048, 448, 16, 28, 1792
HP = 32
DP = H * HP
GR = 4 * DH
TQ = 256
NB = S // TQ
KC = 128
NK = S // KC
NP = H // 2
FH, D2 = F // 2, D // 2
NC = FH // 128
C = D // 4
HALO = 128
EPS = 1e-5
QSCALE = (DH ** -0.5) * math.log2(math.e)
f32, bf16 = jnp.float32, jnp.bfloat16

SDPOS = {2: (0, 0), 3: (D2, FH), 0: (D, 0), 1: (D, FH), 4: (D + D2, 0), 5: (D + D2, FH), 6: (2 * D, 0)}
PLAN = [
    ("wka", "Twka"),
    ("x0 g", "Ka0 Tg"),
    ("x1", "Ka1 S0"),
    ("wkb x2", "Twkb Ka2 S1 Kb0 Kb1 S2 Kb2"),
    ("x3 x4 x5 x6", "K3 S3 T0 K4 S4 T1 K5 S5 S6"),
    ("x7 w1 wv wq", "Tw1 K6 K7 S7 Twv Twq W0 T2 W7 T3 W1 T4 W2 T5 W3 T6 W4 T7 W5 W6"),
    ("w2 wo w3 w4", "Tw2 Two Tw3 Tw4 V0 H0 V1 H1 V2 H2 V3 H3 V4 H4 V5 H5 V6 H6 V7 H7"),
]
SCRATCH = dict(
    gw_r=((D,), bf16),
    sA=((1, S, 2 * TQ), f32), sB=((1, S, 2 * TQ), f32), k_s=((4, S, GR), bf16), vT_s=((DP, S), bf16),
    x_s=((NB, D, TQ), bf16), wqkv_r=((D, 3 * D), bf16), wo_r=((D, D), bf16), w1_r=((D, D), bf16),
    w2_r=((D, D), bf16), w3_r=((D, F), bf16), w4_s=((D + 3 * D2, F), bf16),
    wqkvT_s=((3 * D, D), bf16), so_s=((7, D2, D2), bf16), w1T_s=((D, D), bf16),
    s2_s=((7, D2, D2), bf16), s3_s=((7, FH, D2), bf16),
    kT_s=((NB, D, TQ), bf16), st_s=((NB, 8, TQ), f32),
    h_s=((D, S + 2 * HALO), bf16), hs_s=((NB, D, TQ), bf16), q_s=((D, TQ), bf16),
    oa_s=((NB, 2, C, TQ), bf16), ob_s=((NB, 2, C, TQ), bf16), x1_s=((1, D + 16, TQ), f32),
    sb_s=((1, D2, 7 * 128), bf16), gcol_s=((D + 8, 128), f32), scol_s=((D, 128), f32))


def _gelu(x, half=0.5):
    c = math.sqrt(2.0 / math.pi)
    return half * x * (1.0 + jnp.tanh(c * (x + 0.044715 * (x * x * x))))


def _dot(a, b):
    return jnp.dot(a, b, preferred_element_type=f32)


def _ln_stats(x):
    c0 = x[0:1, :]
    d = x - c0
    m1 = jnp.mean(d, axis=0, keepdims=True)
    m2 = jnp.mean(d * d, axis=0, keepdims=True)
    return c0 + m1, jax.lax.rsqrt(jnp.maximum(m2 - m1 * m1, 0.0) + EPS)


def _sa(a11, a12, a21, a22):
    return [a11 + a22, a21 + a22, a11, a22, a11 + a12, a21 - a11, a12 - a22]


def _sb(b11, b12, b21, b22):
    return [t.astype(bf16) for t in (b11 + b22, b11, b12 - b22, b21 - b11, b22, b11 + b12, b21 + b22)]


def _sc(m):
    return m[0] + m[3] - m[4] + m[6], m[2] + m[4], m[1] + m[3], m[0] - m[1] + m[2] + m[5]


def _quad(x):
    r = x.shape[0] // 2
    return x[:r, :128], x[:r, 128:], x[r:, :128], x[r:, 128:]


def _col(row):
    return jnp.broadcast_to(row, (128, D)).T


def _wide(col):
    return jnp.concatenate([col] * (TQ // 128), axis=1)


def _kernel(x_hbm, wqkv_hbm, wo_hbm, w1_hbm, w2_hbm, w3_hbm, w4T_hbm, gw_hbm, o_hbm,
            gw_r, sA, sB, k_s, vT_s, x_s, wqkv_r, wo_r, w1_r, w2_r, w3_r, w4_s, wqkvT_s, so_s, w1T_s,
            s2_s, s3_s, kT_s, st_s, h_s, hs_s, q_s, oa_s, ob_s, x1_s, sb_s, gcol_s, scol_s,
            sems, osems):
    i = pl.program_id(0)
    zi = jnp.minimum(i, 0)
    cp = pltpu.make_async_copy

    @pl.when(i == 0)
    def _prologue():
        row = jax.lax.broadcasted_iota(jnp.int32, (HP - DH, TQ), 0)
        pad_rows = jnp.where(row == 0, 1.0, 0.0)

        tick = []

        def kproj(b, lo=0, hi=D):
            kT_s[b, lo:hi, :] = _dot(wqkvT_s[D + lo:D + hi, :], x_s[b]).astype(bf16)

        def ktr(b):
            for g in range(4):
                k_s[g, b * TQ:(b + 1) * TQ, :] = kT_s[b, g * GR:(g + 1) * GR, :].T

        def stats(b):
            if b == NB - 1:
                xf = x_s[b].astype(f32)
                mu, rstd = _ln_stats(xf)
                z = jnp.sum(xf * _wide(gcol_s[0:D, :]), axis=0, keepdims=True)
            else:
                c0 = x_s[b, 0:16, :].astype(f32)[0:1, :]
                if not tick:
                    tick.append(jnp.where(i < 0, jnp.broadcast_to(c0[:, :128], (8, 128)), 0.0))
                tot = None
                for r0 in range(0, D, 16):
                    tick[0] = jnp.tanh(jnp.tanh(jnp.tanh(tick[0])))
                    c8 = c0 + jnp.concatenate([tick[0], tick[0]], axis=1)
                    d = x_s[b, r0:r0 + 16, :].astype(f32) - jnp.concatenate([c8, c8], axis=0)
                    part = [t[:8] + t[8:] for t in (d, d * d, d * _wide(gcol_s[r0:r0 + 16, :]))]
                    tot = part if tot is None else [s + t for s, t in zip(tot, part)]
                s1, s2, s3 = [jnp.sum(t, axis=0, keepdims=True) for t in tot]
                m1, m2 = s1 * (1.0 / D), s2 * (1.0 / D)
                mu = c0 + m1
                rstd = jax.lax.rsqrt(jnp.maximum(m2 - m1 * m1, 0.0) + EPS)
                z = s3 + c0 * _wide(gcol_s[D:D + 1, :])
            st_s[b, 0:1, :] = rstd
            st_s[b, 1:2, :] = mu * rstd
            st_s[b, 2:3, :] = jax.nn.sigmoid(z)

        def w1proj(b):
            y = _dot(w1T_s[...], x_s[b])
            pre = y * st_s[b, 0:1, :] - _wide(scol_s[...]) * st_s[b, 1:2, :]
            h_s[:, HALO + b * TQ:HALO + (b + 1) * TQ] = _gelu(pre).astype(bf16)

        def vproj(b):
            v = _dot(wqkvT_s[2 * D:, :], x_s[b])
            for h in range(H):
                vT_s[h * HP:(h + 1) * HP, b * TQ:(b + 1) * TQ] = jnp.concatenate(
                    [v[h * DH:(h + 1) * DH, :], pad_rows], axis=0).astype(bf16)

        def shift(b):
            l0 = HALO + b * TQ
            for g, off in enumerate((-1, 1, -2, 2)):
                hs_s[b, g * C:(g + 1) * C, :] = h_s[g * C:(g + 1) * C, l0 + off:l0 + off + TQ]

        def t_qkv(lo, hi):
            wqkvT_s[lo:hi, :] = wqkv_r[:, lo:hi].T

        def t_w1():
            w1T_s[...] = w1_r[...].T
            scol_s[...] = _col(jnp.sum(w1_r[...].astype(f32), axis=0, keepdims=True))

        def left_ops(w, dst):
            t1, t2 = w[:D2].T.astype(f32), w[D2:].T.astype(f32)
            for k, a in enumerate(_sa(t1[:D2], t2[:D2], t1[D2:], t2[D2:])):
                dst[k] = a.astype(bf16)

        def t_w3():
            for c in range(NC):
                def blk(r, e):
                    return w3_r[r * D2:(r + 1) * D2, e * FH + c * 128:e * FH + (c + 1) * 128].astype(f32)
                for k, a in enumerate(_sa(blk(0, 0), blk(1, 0), blk(0, 1), blk(1, 1))):
                    s3_s[k, c * 128:(c + 1) * 128, :] = a.astype(bf16).T

        def t_w4():
            for r0 in range(0, D2, 16):
                def rows(base):
                    return pl.ds(pl.multiple_of(zi * 16 + base + r0, 16), 16)
                for c0 in range(0, FH, 256):
                    c1 = min(c0 + 256, FH)
                    def blk(r, e):
                        return w4_s[rows(r * D2), e * FH + c0:e * FH + c1].astype(f32)
                    for k, a in enumerate(_sa(blk(0, 0), blk(0, 1), blk(1, 0), blk(1, 1))):
                        if k not in (2, 3):
                            rb, cb = SDPOS[k]
                            w4_s[rows(rb), cb + c0:cb + c1] = a.astype(bf16)

        def t_g():
            gc = _col(gw_r[...].astype(f32).reshape(1, D))
            gcol_s[0:D, :] = gc
            gcol_s[D:D + 1, :] = jnp.sum(gc, axis=0, keepdims=True)

        def cols(lo, n):
            return wqkv_hbm.at[:, pl.ds(lo, n)], wqkv_r.at[:, pl.ds(lo, n)]

        copies = {"g": (gw_hbm, gw_r), "wka": cols(640, 256), "wkb": cols(384, 256),
                  "wv": cols(896, 448), "wq": cols(0, 384),
                  "w1": (w1_hbm, w1_r), "w2": (w2_hbm, w2_r), "wo": (wo_hbm, wo_r), "w3": (w3_hbm, w3_r),
                  "w4": (w4T_hbm, w4_s.at[pl.ds(0, D), :])}
        jobs = {"Twka": functools.partial(t_qkv, 640, 896), "Twkb": functools.partial(t_qkv, 384, 640),
                "Twv": functools.partial(t_qkv, 896, 3 * D), "Twq": functools.partial(t_qkv, 0, 384),
                "Tw1": t_w1,
                "Tw2": lambda: left_ops(w2_r[...], s2_s), "Two": lambda: left_ops(wo_r[...], so_s),
                "Tw3": t_w3, "Tw4": t_w4, "Tg": t_g}
        for b in range(NB):
            jobs["Ka%d" % b] = functools.partial(kproj, b, 640 - D, D)
            jobs["Kb%d" % b] = functools.partial(kproj, b, 0, 640 - D)
            copies["x%d" % b] = (x_hbm.at[:, pl.ds(b * TQ, TQ)], x_s.at[b])
            for nm, fn in (("K", kproj), ("T", ktr), ("S", stats), ("W", w1proj), ("V", vproj), ("H", shift)):
                jobs["%s%d" % (nm, b)] = functools.partial(fn, b)

        grp = [[cp(*copies[n], sems.at[k]) for n in g.split()] for k, (g, _) in enumerate(PLAN)]
        for g in grp:
            for c in g:
                c.start()
        h_s[:, 0:HALO] = jnp.zeros((D, HALO), bf16)
        h_s[:, HALO + S:] = jnp.zeros((D, HALO), bf16)
        for k, (_, js) in enumerate(PLAN):
            for c in grp[k]:
                c.wait()
            tick.clear()
            for j in js.split():
                jobs[j]()

    xb = x_s[i]
    q_s[...] = (_dot(wqkvT_s[0:D, :], xb) * QSCALE).astype(bf16)
    gt = st_s[i, 2:3, :]

    hb = _sb(*_quad(hs_s[i].astype(f32)))
    c11, c12, c21, c22 = _sc([_dot(s2_s[k], hb[k]) for k in range(7)])
    x1 = xb.astype(f32) + jnp.concatenate(
        [jnp.concatenate([c11, c12], axis=1), jnp.concatenate([c21, c22], axis=1)], axis=0)
    x1_s[zi, 0:D, :] = x1
    mu, rstd = _ln_stats(x1)
    mu = jnp.broadcast_to(mu, (16, TQ))
    rstd = jnp.broadcast_to(rstd, (16, TQ))
    for r0 in range(0, D2, 16):
        def ld(base):
            return x1_s[0, pl.ds(pl.multiple_of(zi * 16 + base + r0, 16), 16), :]
        t, b = (ld(0) - mu) * rstd, (ld(D2) - mu) * rstd
        ops = _sb(t[:, :128], t[:, 128:], b[:, :128], b[:, 128:])
        for k in range(7):
            sb_s[zi, r0:r0 + 16, k * 128:(k + 1) * 128] = ops[k]
        x1_s[0, pl.ds(pl.multiple_of(zi * 16 + D + (r0 % 32) // 2, 8), 8), 0:128] = t[:8, :128] + b[:8, 128:]

    grow = jax.lax.broadcasted_iota(jnp.int32, (GR, TQ), 0)
    sbuf = (sA, sB)
    qm, pmax, mx, acc = [None] * NP, [None] * NP, [None] * NP, [None] * H

    def qk(p, c):
        g = p // 2
        if c == 0:
            qg = q_s[g * GR:(g + 1) * GR, :]
            z = jnp.zeros_like(qg)
            j = (2 * p) % 4
            qm[p] = jnp.concatenate(
                [jnp.where((grow >= jj * DH) & (grow < (jj + 1) * DH), qg, z) for jj in (j, j + 1)], axis=1)
        s = _dot(k_s[g, c * KC:(c + 1) * KC, :], qm[p])
        sbuf[p % 2][zi, c * KC:(c + 1) * KC, :] = s
        pm = jnp.max(s.reshape(KC // 8, 8, 2 * TQ), axis=0)
        pmax[p] = pm if c == 0 else jnp.maximum(pmax[p], pm)
        if c == NK - 1:
            mx[p] = jnp.max(pmax[p], axis=0, keepdims=True)

    def sm(p, c):
        e, cc = c % 2, c // 2
        h = 2 * p + e
        rows = slice(cc * 2 * KC, (cc + 1) * 2 * KC)
        pp = jnp.exp2(sbuf[p % 2][zi, rows, e * TQ:(e + 1) * TQ] - mx[p][:, e * TQ:(e + 1) * TQ]).astype(bf16)
        d = _dot(vT_s[h * HP:(h + 1) * HP, rows], pp)
        acc[h] = d if cc == 0 else acc[h] + d
        if cc == NK // 2 - 1:
            acc[h] = (acc[h] * (1.0 / acc[h][DH:DH + 1, :]))[:DH]

    um = [[None] * 7 for _ in range(NC)]
    tb, dm, last, ob = [None] * NC, [None] * 7, [None] * 7, []
    hg = 0.5 * (1.0 - gt)
    hq = (hg[:, :128], hg[:, 128:]) * 2

    def up(c, k):
        um[c][k] = _dot(s3_s[k, c * 128:(c + 1) * 128, :], sb_s[zi, :, k * 128:(k + 1) * 128])
        if k == 5:
            tb[c] = _sb(*[_gelu(t, hh) for t, hh in zip(_sc(um[c]), hq)])

    def down(c, k):
        rb, cb = SDPOS[k]
        d = _dot(w4_s[rb:rb + D2, cb + c * 128:cb + (c + 1) * 128], tb[c][k])
        if c == NC - 1 and k in (1, 2, 5, 6):
            last[k] = d
        else:
            dm[k] = d if c == 0 else dm[k] + d

    def oproj(_, k):
        if not ob:
            ob.extend(_sb(*_quad(jnp.concatenate(acc, axis=0) * gt)))
        dm[k] = dm[k] + _dot(so_s[k], ob[k])

    dots = []
    for c in range(NC):
        dots += [(up, c, k) for k in (0, 3, 4, 6, 2, 1, 5)]
        if c >= 1:
            dots += [(down, c - 1, k) for k in range(7)]
    dots += [(oproj, 0, k) for k in range(7)]
    dots += [(down, NC - 1, k) for k in (0, 3, 4, 1, 2, 5, 6)]

    for n in range(NP * NK):
        qk(n // NK, n % NK)
        if n >= NK:
            sm(n // NK - 1, n % NK)
    for n, (fn, c, k) in enumerate(dots):
        fn(c, k)
        if n % 3 == 2 and n // 3 < NK:
            sm(NP - 1, n // 3)

    base = [xg + cc for xg, cc in zip(_quad(x1_s[zi, 0:D, :] * (1.0 - gt)), _sc(dm))]
    top = jnp.concatenate([base[0] + last[6], base[1] + last[2]], axis=1).astype(bf16)
    bot = jnp.concatenate([base[2] + last[1], base[3] - last[1] + last[2] + last[5]], axis=1).astype(bf16)
    col0 = pl.multiple_of(i * TQ, TQ)
    for n, buf in enumerate((oa_s, ob_s)):
        buf[i, 0] = top[n * C:(n + 1) * C]
        buf[i, 1] = bot[n * C:(n + 1) * C]
        for e in range(2):
            cp(buf.at[i, e], o_hbm.at[pl.ds(e * D2 + n * C, C), pl.ds(col0, TQ)], osems.at[n]).start()

    @pl.when(i == NB - 1)
    def _drain():
        for n, buf in enumerate((oa_s, ob_s)):
            cp(buf, buf, osems.at[n]).wait()


@jax.jit
def pallas_gated_mix__mha_block__mixer_s_mlp__prompt_kernel(
    A_x: jax.Array,
    A_wqkv: jax.Array,
    A_wo: jax.Array,
    B_x: jax.Array,
    B_w1: jax.Array,
    B_w2: jax.Array,
    B_w3: jax.Array,
    B_w4: jax.Array,
    gate_w: jax.Array,
):
    args = (A_x.reshape(S, D).T, A_wqkv, A_wo, B_w1, B_w2, B_w3, B_w4.T, gate_w)
    extra = {}
    if hasattr(pltpu.CompilerParams, "disable_semaphore_checks"):
        extra["disable_semaphore_checks"] = True
    out_t = pl.pallas_call(
        _kernel,
        grid=(NB,),
        in_specs=[pl.BlockSpec(memory_space=pl.ANY)] * len(args),
        out_specs=pl.BlockSpec(memory_space=pl.ANY),
        out_shape=jax.ShapeDtypeStruct((D, S), bf16),
        scratch_shapes=[pltpu.VMEM(*v) for v in SCRATCH.values()]
        + [pltpu.SemaphoreType.DMA((len(PLAN),)), pltpu.SemaphoreType.DMA((2,))],
        compiler_params=pltpu.CompilerParams(
            dimension_semantics=("arbitrary",), vmem_limit_bytes=100 * 1024 * 1024,
            disable_bounds_checks=True, **extra),
    )(*args)
    return out_t.T.reshape(1, S, D)
```

```python
import functools
import math

import jax
import jax.numpy as jnp
import jax.experimental.pallas as pl
import jax.experimental.pallas.tpu as pltpu

S, D, H, DH, F = 2048, 448, 16, 28, 1792
HP = 32
DP = H * HP
GR = 4 * DH
TQ = 256
NB = S // TQ
KC = 128
NK = S // KC
NP = H // 2
FH, D2 = F // 2, D // 2
NC = FH // 128
C = D // 4
HALO = 128
NVP = (64, 32, 64, 64, 64, 64, 64, 64)
VG = 32
NS = 14
EPS = 1e-5
QSCALE = (DH ** -0.5) * math.log2(math.e)
f32, bf16 = jnp.float32, jnp.bfloat16

SDPOS = {2: (0, 0), 3: (D2, FH), 0: (D, 0), 1: (D, FH), 4: (D + D2, 0), 5: (D + D2, FH), 6: (2 * D, 0)}
PLAN = [
    ("wka", "Twka"),
    ("x0 g", "Ka0 Tg"),
    ("x1", "Ka1 S0"),
    ("wkb x2", "Twkb Ka2 S1 Kb0 Kb1 S2 Kb2"),
    ("x3 x4 x5 x6", "K3 S3 T0 K4 S4 T1 K5 S5 S6"),
    ("x7 w1 wv wq", "Tw1 K6 K7 S7 Twv Twq W0 T2 W7 T3 W1 T4 W2 T5 W3 T6 W4 T7 W5 W6"),
    ("w2 wo w3 w4", "Tw2 Two Tw3 Tw4 V0 H0 V1 H1 V2 H2 V3 H3 V4 H4 V5 H5 V6 H6 V7 H7"),
]
SCRATCH = dict(
    gw_r=((D,), bf16),
    sA=((1, S, 2 * TQ), f32), sB=((1, S, 2 * TQ), f32), k_s=((4, S, GR), bf16), vT_s=((DP, S), bf16),
    x_s=((NB, D, TQ), bf16), wqkv_r=((D, 3 * D), bf16), wo_r=((D, D), bf16), w1_r=((D, D), bf16),
    w2_r=((D, D), bf16), w3_r=((D, F), bf16), w4_s=((D + 3 * D2, F), bf16),
    wqkvT_s=((3 * D, D), bf16), so_s=((7, D2, D2), bf16), w1T_s=((D, D), bf16),
    s2_s=((7, D2, D2), bf16), s3_s=((7, FH, D2), bf16),
    kT_s=((NB, D, TQ), bf16), st_s=((NB, 8, TQ), f32),
    h_s=((D, S + 2 * HALO), bf16), hs_s=((NB, D, TQ), bf16), q_s=((D, TQ), bf16),
    oa_s=((NB, 2, C, TQ), bf16), ob_s=((NB, 2, C, TQ), bf16), x1_s=((1, D + 16, TQ), f32),
    qf_s=((1, 2, D, 128), f32),
    sb_s=((1, D2, 7 * 128), bf16), gcol_s=((D + 8, 128), f32), scol_s=((D, 128), f32))


def _gelu(x, half=0.5):
    c = math.sqrt(2.0 / math.pi)
    return half * x * (1.0 + jnp.tanh(c * (x + 0.044715 * (x * x * x))))


def _dot(a, b):
    return jnp.dot(a, b, preferred_element_type=f32)


def _ln_stats(x):
    c0 = x[0:1, :]
    d = x - c0
    m1 = jnp.mean(d, axis=0, keepdims=True)
    m2 = jnp.mean(d * d, axis=0, keepdims=True)
    return c0 + m1, jax.lax.rsqrt(jnp.maximum(m2 - m1 * m1, 0.0) + EPS)


def _sa(a11, a12, a21, a22):
    return [a11 + a22, a21 + a22, a11, a22, a11 + a12, a21 - a11, a12 - a22]


def _sb(b11, b12, b21, b22):
    return [t.astype(bf16) for t in (b11 + b22, b11, b12 - b22, b21 - b11, b22, b11 + b12, b21 + b22)]


def _sc(m):
    return m[0] + m[3] - m[4] + m[6], m[2] + m[4], m[1] + m[3], m[0] - m[1] + m[2] + m[5]


def _quad(x):
    r = x.shape[0] // 2
    return x[:r, :128], x[:r, 128:], x[r:, :128], x[r:, 128:]


def _col(row):
    return jnp.broadcast_to(row, (128, D)).T


def _wide(col):
    return jnp.concatenate([col] * (TQ // 128), axis=1)


def _kernel(x_hbm, wqkv_hbm, wo_hbm, w1_hbm, w2_hbm, w3_hbm, w4T_hbm, gw_hbm, o_hbm,
            gw_r, sA, sB, k_s, vT_s, x_s, wqkv_r, wo_r, w1_r, w2_r, w3_r, w4_s, wqkvT_s, so_s, w1T_s,
            s2_s, s3_s, kT_s, st_s, h_s, hs_s, q_s, oa_s, ob_s, x1_s, qf_s, sb_s, gcol_s, scol_s,
            sems, osems):
    i = pl.program_id(0)
    zi = jnp.minimum(i, 0)
    cp = pltpu.make_async_copy

    @pl.when(i == 0)
    def _prologue():
        row = jax.lax.broadcasted_iota(jnp.int32, (HP - DH, TQ), 0)
        pad_rows = jnp.where(row == 0, 1.0, 0.0)
        tick = []

        def kproj(b, lo=0, hi=D):
            kT_s[b, lo:hi, :] = _dot(wqkvT_s[D + lo:D + hi, :], x_s[b]).astype(bf16)

        def ktr(b):
            for g in range(4):
                k_s[g, b * TQ:(b + 1) * TQ, :] = kT_s[b, g * GR:(g + 1) * GR, :].T

        def stats(b):
            if b == NB - 1:
                xf = x_s[b].astype(f32)
                mu, rstd = _ln_stats(xf)
                z = jnp.sum(xf * _wide(gcol_s[0:D, :]), axis=0, keepdims=True)
            else:
                c0 = x_s[b, 0:16, :].astype(f32)[0:1, :]
                if not tick:
                    tick.append(jnp.where(i < 0, jnp.broadcast_to(c0[:, :128], (8, 128)), 0.0))
                tot = None
                for r0 in range(0, D, 16):
                    tick[0] = jnp.tanh(jnp.tanh(jnp.tanh(tick[0])))
                    c8 = c0 + jnp.concatenate([tick[0], tick[0]], axis=1)
                    d = x_s[b, r0:r0 + 16, :].astype(f32) - jnp.concatenate([c8, c8], axis=0)
                    part = [t[:8] + t[8:] for t in (d, d * d, d * _wide(gcol_s[r0:r0 + 16, :]))]
                    tot = part if tot is None else [s + t for s, t in zip(tot, part)]
                s1, s2, s3 = [jnp.sum(t, axis=0, keepdims=True) for t in tot]
                m1, m2 = s1 * (1.0 / D), s2 * (1.0 / D)
                mu = c0 + m1
                rstd = jax.lax.rsqrt(jnp.maximum(m2 - m1 * m1, 0.0) + EPS)
                z = s3 + c0 * _wide(gcol_s[D:D + 1, :])
            st_s[b, 0:1, :] = rstd
            st_s[b, 1:2, :] = mu * rstd
            st_s[b, 2:3, :] = jax.nn.sigmoid(z)

        def w1proj(b):
            y = _dot(w1T_s[...], x_s[b])
            pre = y * st_s[b, 0:1, :] - _wide(scol_s[...]) * st_s[b, 1:2, :]
            h_s[:, HALO + b * TQ:HALO + (b + 1) * TQ] = _gelu(pre).astype(bf16)

        def vproj(b):
            v = _dot(wqkvT_s[2 * D:, :], x_s[b])
            for h in range(H):
                vT_s[h * HP:(h + 1) * HP, b * TQ:(b + 1) * TQ] = jnp.concatenate(
                    [v[h * DH:(h + 1) * DH, :], pad_rows], axis=0).astype(bf16)

        def shift(b):
            l0 = HALO + b * TQ
            for g, off in enumerate((-1, 1, -2, 2)):
                hs_s[b, g * C:(g + 1) * C, :] = h_s[g * C:(g + 1) * C, l0 + off:l0 + off + TQ]

        def t_qkv(lo, hi):
            wqkvT_s[lo:hi, :] = wqkv_r[:, lo:hi].T

        def t_w1():
            w1T_s[...] = w1_r[...].T
            scol_s[...] = _col(jnp.sum(w1_r[...].astype(f32), axis=0, keepdims=True))

        def left_ops(w, dst):
            t1, t2 = w[:D2].T.astype(f32), w[D2:].T.astype(f32)
            for k, a in enumerate(_sa(t1[:D2], t2[:D2], t1[D2:], t2[D2:])):
                dst[k] = a.astype(bf16)

        def t_w3():
            for c in range(NC):
                def blk(r, e):
                    return w3_r[r * D2:(r + 1) * D2, e * FH + c * 128:e * FH + (c + 1) * 128].astype(f32)
                for k, a in enumerate(_sa(blk(0, 0), blk(1, 0), blk(0, 1), blk(1, 1))):
                    s3_s[k, c * 128:(c + 1) * 128, :] = a.astype(bf16).T

        def t_w4():
            for r0 in range(0, D2, 16):
                def rows(base):
                    return pl.ds(pl.multiple_of(zi * 16 + base + r0, 16), 16)
                for c0 in range(0, FH, 256):
                    c1 = min(c0 + 256, FH)
                    def blk(r, e):
                        return w4_s[rows(r * D2), e * FH + c0:e * FH + c1].astype(f32)
                    for k, a in enumerate(_sa(blk(0, 0), blk(0, 1), blk(1, 0), blk(1, 1))):
                        if k not in (2, 3):
                            rb, cb = SDPOS[k]
                            w4_s[rows(rb), cb + c0:cb + c1] = a.astype(bf16)

        def t_g():
            gc = _col(gw_r[...].astype(f32).reshape(1, D))
            gcol_s[0:D, :] = gc
            gcol_s[D:D + 1, :] = jnp.sum(gc, axis=0, keepdims=True)

        def cols(lo, n):
            return wqkv_hbm.at[:, pl.ds(lo, n)], wqkv_r.at[:, pl.ds(lo, n)]

        copies = {"g": (gw_hbm, gw_r), "wka": cols(640, 256), "wkb": cols(384, 256),
                  "wv": cols(896, 448), "wq": cols(0, 384),
                  "w1": (w1_hbm, w1_r), "w2": (w2_hbm, w2_r), "wo": (wo_hbm, wo_r), "w3": (w3_hbm, w3_r),
                  "w4": (w4T_hbm, w4_s.at[pl.ds(0, D), :])}
        jobs = {"Twka": functools.partial(t_qkv, 640, 896), "Twkb": functools.partial(t_qkv, 384, 640),
                "Twv": functools.partial(t_qkv, 896, 3 * D), "Twq": functools.partial(t_qkv, 0, 384),
                "Tw1": t_w1,
                "Tw2": lambda: left_ops(w2_r[...], s2_s), "Two": lambda: left_ops(wo_r[...], so_s),
                "Tw3": t_w3, "Tw4": t_w4, "Tg": t_g}
        for b in range(NB):
            jobs["Ka%d" % b] = functools.partial(kproj, b, 640 - D, D)
            jobs["Kb%d" % b] = functools.partial(kproj, b, 0, 640 - D)
            copies["x%d" % b] = (x_hbm.at[:, pl.ds(b * TQ, TQ)], x_s.at[b])
            for nm, fn in (("K", kproj), ("T", ktr), ("S", stats), ("W", w1proj), ("V", vproj), ("H", shift)):
                jobs["%s%d" % (nm, b)] = functools.partial(fn, b)

        grp = [[cp(*copies[n], sems.at[k]) for n in g.split()] for k, (g, _) in enumerate(PLAN)]
        for g in grp:
            for c in g:
                c.start()
        h_s[:, 0:HALO] = jnp.zeros((D, HALO), bf16)
        h_s[:, HALO + S:] = jnp.zeros((D, HALO), bf16)
        for k, (_, js) in enumerate(PLAN):
            for c in grp[k]:
                c.wait()
            tick.clear()
            for j in js.split():
                jobs[j]()

    xb = x_s[i]
    qb = (_dot(wqkvT_s[0:D, :], xb) * QSCALE).astype(bf16)
    q_s[...] = qb
    for t in range(2):
        qf_s[zi, t] = qb[:, t * 128:(t + 1) * 128].astype(f32)
    gt = st_s[i, 2:3, :]

    hb = _sb(*_quad(hs_s[i].astype(f32)))
    c11, c12, c21, c22 = _sc([_dot(s2_s[k], hb[k]) for k in range(7)])
    x1 = xb.astype(f32) + jnp.concatenate(
        [jnp.concatenate([c11, c12], axis=1), jnp.concatenate([c21, c22], axis=1)], axis=0)
    x1_s[zi, 0:D, :] = x1
    mu, rstd = _ln_stats(x1)
    mu = jnp.broadcast_to(mu, (16, TQ))
    rstd = jnp.broadcast_to(rstd, (16, TQ))
    for r0 in range(0, D2, 16):
        def ld(base):
            return x1_s[0, pl.ds(pl.multiple_of(zi * 16 + base + r0, 16), 16), :]
        t, b = (ld(0) - mu) * rstd, (ld(D2) - mu) * rstd
        ops = _sb(t[:, :128], t[:, 128:], b[:, :128], b[:, 128:])
        for k in range(7):
            sb_s[zi, r0:r0 + 16, k * 128:(k + 1) * 128] = ops[k]
        x1_s[0, pl.ds(pl.multiple_of(zi * 16 + D + (r0 % 32) // 2, 8), 8), 0:128] = t[:8, :128] + b[:8, 128:]

    grow = jax.lax.broadcasted_iota(jnp.int32, (GR, TQ), 0)
    sbuf = (sA, sB)
    qm, pmax, mx, acc = [None] * NP, [None] * NP, [None] * NP, [None] * H
    va, pend = [None], []

    def qk(p, c):
        g = p // 2
        if c == 0:
            qg = q_s[g * GR:(g + 1) * GR, :]
            z = jnp.zeros_like(qg)
            j = (2 * p) % 4
            qm[p] = jnp.concatenate(
                [jnp.where((grow >= jj * DH) & (grow < (jj + 1) * DH), qg, z) for jj in (j, j + 1)], axis=1)
        s = raw = _dot(k_s[g, c * KC:min((c + 1) * KC, S - NVP[p]), :], qm[p])
        n = s.shape[0]
        for j, pv in pend:
            r = j * 64 + 32
            blk = jnp.concatenate([jnp.where(i < 0, pv, s[r:r + VG, :TQ]), s[r:r + VG, TQ:]], axis=1)
            s = jnp.concatenate([s[:r], blk] + ([s[r + VG:]] if r + VG < n else []), axis=0)
        pend.clear()
        sbuf[p % 2][zi, c * KC:c * KC + n, :] = s
        pm = jnp.max(s.reshape(n // 8, 8, 2 * TQ), axis=0)
        pmax[p] = pm if c == 0 else jnp.maximum(pmax[p], pm)
        items = [(e, r0, dd) for e in range(2) for r0 in range(S - NVP[p], S, VG) for dd in range(DH)]
        per = len(items) // (2 * NS)
        for j in range(2 if c < NS else 0):
            batch = items[(2 * c + j) * per:(2 * c + j + 1) * per]
            e, r0 = batch[0][:2]
            h = 2 * p + e
            zero = jnp.where(i < 0, raw[j * 64:j * 64 + 8, :GR], 0.0)
            kf = k_s[g, r0:r0 + VG, :].astype(f32) + jnp.concatenate([zero] * (VG // 8), axis=0)
            for _, _, dd in batch:
                o, r = (h % 4) * DH + dd, h * DH + dd
                kb = jnp.broadcast_to(kf[:, o:o + 1], (VG, 128))
                u = jnp.concatenate(
                    [kb * qf_s[zi, t, r // 8 * 8:r // 8 * 8 + 8, :][r % 8:r % 8 + 1, :] for t in range(2)], axis=1)
                va[0] = u if dd == 0 else va[0] + u
            if dd == DH - 1:
                sbuf[p % 2][zi, r0:r0 + VG, e * TQ:(e + 1) * TQ] = va[0]
                vm = jnp.max(va[0].reshape(VG // 8, 8, TQ), axis=0)
                pa, pb = pmax[p][:, :TQ], pmax[p][:, TQ:]
                pmax[p] = jnp.concatenate(
                    [jnp.maximum(pa, vm), pb] if e == 0 else [pa, jnp.maximum(pb, vm)], axis=1)
            pend.append((j, va[0]))
        if c == NK - 1:
            mx[p] = jnp.max(pmax[p], axis=0, keepdims=True)

    def sm(p, c):
        e, cc = c % 2, c // 2
        h = 2 * p + e
        rows = slice(cc * 2 * KC, (cc + 1) * 2 * KC)
        pp = jnp.exp2(sbuf[p % 2][zi, rows, e * TQ:(e + 1) * TQ] - mx[p][:, e * TQ:(e + 1) * TQ]).astype(bf16)
        d = _dot(vT_s[h * HP:(h + 1) * HP, rows], pp)
        acc[h] = d if cc == 0 else acc[h] + d
        if cc == NK // 2 - 1:
            acc[h] = (acc[h] * (1.0 / acc[h][DH:DH + 1, :]))[:DH]

    um = [[None] * 7 for _ in range(NC)]
    tb, dm, last, ob = [None] * NC, [None] * 7, [None] * 7, []
    hg = 0.5 * (1.0 - gt)
    hq = (hg[:, :128], hg[:, 128:]) * 2

    def up(c, k):
        um[c][k] = _dot(s3_s[k, c * 128:(c + 1) * 128, :], sb_s[zi, :, k * 128:(k + 1) * 128])
        if k == 5:
            tb[c] = _sb(*[_gelu(t, hh) for t, hh in zip(_sc(um[c]), hq)])

    def down(c, k):
        rb, cb = SDPOS[k]
        d = _dot(w4_s[rb:rb + D2, cb + c * 128:cb + (c + 1) * 128], tb[c][k])
        if c == NC - 1 and k in (1, 2, 5, 6):
            last[k] = d
        else:
            dm[k] = d if c == 0 else dm[k] + d

    def oproj(_, k):
        if not ob:
            ob.extend(_sb(*_quad(jnp.concatenate(acc, axis=0) * gt)))
        dm[k] = dm[k] + _dot(so_s[k], ob[k])

    dots = []
    for c in range(NC):
        dots += [(up, c, k) for k in (0, 3, 4, 6, 2, 1, 5)]
        if c >= 1:
            dots += [(down, c - 1, k) for k in range(7)]
    dots += [(oproj, 0, k) for k in range(7)]
    dots += [(down, NC - 1, k) for k in (0, 3, 4, 1, 2, 5, 6)]

    for n in range(NP * NK):
        qk(n // NK, n % NK)
        if n >= NK:
            sm(n // NK - 1, n % NK)
    for n, (fn, c, k) in enumerate(dots):
        fn(c, k)
        if n % 3 == 2 and n // 3 < NK:
            sm(NP - 1, n // 3)

    base = [xg + cc for xg, cc in zip(_quad(x1_s[zi, 0:D, :] * (1.0 - gt)), _sc(dm))]
    top = jnp.concatenate([base[0] + last[6], base[1] + last[2]], axis=1).astype(bf16)
    bot = jnp.concatenate([base[2] + last[1], base[3] - last[1] + last[2] + last[5]], axis=1).astype(bf16)
    col0 = pl.multiple_of(i * TQ, TQ)
    for n, buf in enumerate((oa_s, ob_s)):
        buf[i, 0] = top[n * C:(n + 1) * C]
        buf[i, 1] = bot[n * C:(n + 1) * C]
        for e in range(2):
            cp(buf.at[i, e], o_hbm.at[pl.ds(e * D2 + n * C, C), pl.ds(col0, TQ)], osems.at[n]).start()

    @pl.when(i == NB - 1)
    def _drain():
        for n, buf in enumerate((oa_s, ob_s)):
            cp(buf, buf, osems.at[n]).wait()


@jax.jit
def pallas_gated_mix__mha_block__mixer_s_mlp__prompt_kernel(
    A_x: jax.Array,
    A_wqkv: jax.Array,
    A_wo: jax.Array,
    B_x: jax.Array,
    B_w1: jax.Array,
    B_w2: jax.Array,
    B_w3: jax.Array,
    B_w4: jax.Array,
    gate_w: jax.Array,
):
    args = (A_x.reshape(S, D).T, A_wqkv, A_wo, B_w1, B_w2, B_w3, B_w4.T, gate_w)
    extra = {}
    if hasattr(pltpu.CompilerParams, "disable_semaphore_checks"):
        extra["disable_semaphore_checks"] = True
    out_t = pl.pallas_call(
        _kernel,
        grid=(NB,),
        in_specs=[pl.BlockSpec(memory_space=pl.ANY)] * len(args),
        out_specs=pl.BlockSpec(memory_space=pl.ANY),
        out_shape=jax.ShapeDtypeStruct((D, S), bf16),
        scratch_shapes=[pltpu.VMEM(*v) for v in SCRATCH.values()]
        + [pltpu.SemaphoreType.DMA((len(PLAN),)), pltpu.SemaphoreType.DMA((2,))],
        compiler_params=pltpu.CompilerParams(
            dimension_semantics=("arbitrary",), vmem_limit_bytes=100 * 1024 * 1024,
            disable_bounds_checks=True, **extra),
    )(*args)
    return out_t.T.reshape(1, S, D)
```
